```python
import jax
import jax.numpy as jnp

def _softmax(x, axis=-1):
    return jax.nn.softmax(x, axis=axis)
def _gelu(x):
    return jax.nn.gelu(x, approximate=True)
def _silu(x):
    return jax.nn.silu(x)
def _sigmoid(x):
    return jax.nn.sigmoid(x)
def _layernorm(x, axis=-1, eps=1e-5):
    m = jnp.mean(x, axis=axis, keepdims=True)
    v = jnp.var(x, axis=axis, keepdims=True)
    return (x - m) / jnp.sqrt(v + eps)
def _scatter_add(tgt, idx, src, axis=0):
    return tgt.at[idx].add(src)
def _segment_sum(src, seg, n):
    return jax.ops.segment_sum(src, seg, n)
class _Rng:
    def __init__(self, key):
        self._k = key
    def _next(self):
        self._k, sub = jax.random.split(self._k)
        return sub
    def normal(self, shape):
        return jax.random.normal(self._next(), shape, dtype=jnp.bfloat16)
    def randint(self, lo, hi, shape):
        return jax.random.randint(self._next(), shape, lo, hi, dtype=jnp.int32)
    def uniform(self, shape, lo=0.0, hi=1.0):
        return jax.random.uniform(self._next(), shape, jnp.bfloat16, lo, hi)
    def permutation(self, n):
        return jax.random.permutation(self._next(), n)


kernel_name = 'standalone__modern_conv_block_slak__vision'

def setup_inputs():
    _rng = _Rng(jax.random.key(int.from_bytes(__import__("os").urandom(4), "little")))
    _w = (lambda a: (lambda t: t.astype(jnp.bfloat16) if jnp.issubdtype(t.dtype, jnp.floating) else t)(jnp.asarray(a)))
    H = W = 384
    C = 384
    K = 1
    return {
        "x": _w((lambda *s: _rng.normal(s) * 0.05)(1, H, W, C)),
        "dw": _w((lambda *s: _rng.normal(s) * 0.05)(K, K, C)),
        "w1": _w((lambda *s: _rng.normal(s) * 0.05)(C, 4 * C)),
        "w2": _w((lambda *s: _rng.normal(s) * 0.05)(4 * C, C)),
        "grn_g": _w((lambda *s: _rng.normal(s) * 0.05)(4 * C)),
        "grn_b": _w((lambda *s: _rng.normal(s) * 0.05)(4 * C)),
    }

def reference(x, dw, w1, w2, grn_g, grn_b):
    B, H, W, C = x.shape
    K = dw.shape[0]
    pad = K // 2
    xp = jnp.pad(x, ((0,0),(pad,pad),(pad,pad),(0,0)))
    out = jnp.zeros_like(x)
    for i in range(K):
        for j in range(K):
            out = out + xp[:, i:i+H, j:j+W, :] * dw[i, j][None, None, None, :]
    h = _layernorm(out, axis=-1)
    h = _gelu(h @ w1)
    gx = jnp.sqrt((h * h).sum(axis=(1, 2), keepdims=True) + 1e-6)
    nx = gx / (gx.mean(axis=-1, keepdims=True) + 1e-6)
    h = grn_g[None, None, None, :] * (h * nx) + grn_b[None, None, None, :] + h
    return x + h @ w2
```

```python
import functools
import numpy as np
import jax
import jax.numpy as jnp
import jax.experimental.pallas as pl
import jax.experimental.pallas.tpu as pltpu

F32 = jnp.float32
BF16 = jnp.bfloat16
C0 = float(np.sqrt(2.0 / np.pi))
C1 = float(np.sqrt(2.0 / np.pi) * 0.044715)


def make(TM=1024, TC=192, M1=256, N1=512, M2=256, NBUF=2, vmem_mb=126):
    TH = TM - TC

    def kernel(x_hbm, dw_ref, w1_ref, w2_ref, g_ref, b_ref, o_hbm, h_hbm,
               xbuf, hbuf, obuf, hcache, w2s, ssq, sem_x, sem_h, sem_o):
        N, C = x_hbm.shape
        D = w1_ref.shape[1]
        NB = N // TM

        def x_copy(i, slot):
            return pltpu.make_async_copy(x_hbm.at[pl.ds(i * TM, TM)], xbuf.at[slot], sem_x.at[slot])

        def h_out(i, slot):
            return pltpu.make_async_copy(hbuf.at[slot], h_hbm.at[pl.ds(i * TH, TH)], sem_h.at[slot])

        def h_in(i, slot):
            return pltpu.make_async_copy(h_hbm.at[pl.ds(i * TH, TH)], hbuf.at[slot], sem_h.at[slot])

        def o_copy(i, slot):
            return pltpu.make_async_copy(obuf.at[slot], o_hbm.at[pl.ds(i * TM, TM)], sem_o.at[slot])

        ssq[...] = jnp.zeros_like(ssq)
        for s in range(NBUF - 1):
            x_copy(s, s).start()

        def h_store(i, slot, r0, m, c0, n, val):
            if r0 + m <= TC:
                hcache[i, r0:r0 + m, c0:c0 + n] = val
            elif r0 >= TC:
                hbuf[slot, r0 - TC:r0 - TC + m, c0:c0 + n] = val
            else:
                k = TC - r0
                hcache[i, r0:TC, c0:c0 + n] = val[:k]
                hbuf[slot, 0:m - k, c0:c0 + n] = val[k:]

        def h_load(i, slot, r0, m):
            if r0 + m <= TC:
                return hcache[i, r0:r0 + m, :]
            elif r0 >= TC:
                return hbuf[slot, r0 - TC:r0 - TC + m, :]
            else:
                k = TC - r0
                return jnp.concatenate([hcache[i, r0:TC, :], hbuf[slot, 0:m - k, :]], axis=0)

        def p1(i, carry):
            slot = i % NBUF

            @pl.when(i + NBUF - 1 < NB)
            def _():
                x_copy(i + NBUF - 1, (i + NBUF - 1) % NBUF).start()

            x_copy(i, slot).wait()

            @pl.when(i >= NBUF)
            def _():
                h_out(i - NBUF, slot).wait()

            dw = dw_ref[...].astype(F32)
            for r0 in range(0, TM, M1):
                xv = xbuf[slot, r0:r0 + M1, :].astype(F32) * dw
                mu = jnp.mean(xv, axis=-1, keepdims=True)
                xc = xv - mu
                var = jnp.mean(xc * xc, axis=-1, keepdims=True)
                a = (xc * jax.lax.rsqrt(var + 1e-5)).astype(BF16)
                for c0 in range(0, D, N1):
                    z = jnp.dot(a, w1_ref[:, c0:c0 + N1], preferred_element_type=F32)
                    u = z * (C0 + C1 * (z * z))
                    hz = 0.5 * z
                    hv = hz + hz * jnp.tanh(u)
                    sq = hv * hv
                    ssq[:, c0:c0 + N1] += jnp.sum(sq.reshape(M1 // 8, 8, N1), axis=0)
                    h_store(i, slot, r0, M1, c0, N1, hv.astype(BF16))
            h_out(i, slot).start()
            return carry

        jax.lax.fori_loop(0, NB, p1, 0)
        for s in range(NBUF):
            i = NB - NBUF + s
            h_out(i, i % NBUF).wait()

        for s in range(NBUF - 1):
            x_copy(s, s).start()
            h_in(s, s).start()

        gx = jnp.sqrt(jnp.sum(ssq[...], axis=0, keepdims=True) + 1e-6)
        nx = gx / (jnp.mean(gx, axis=-1, keepdims=True) + 1e-6)
        sc = 1.0 + g_ref[...].astype(F32) * nx
        scT = jnp.broadcast_to(sc, (128, D)).T
        for c0 in range(0, C, 128):
            w2s[:, c0:c0 + 128] = (w2_ref[:, c0:c0 + 128].astype(F32) * scT).astype(BF16)
        bias = jnp.dot(jnp.broadcast_to(b_ref[...], (16, D)), w2_ref[...], preferred_element_type=F32)[0:1]

        def p2(i, carry):
            slot = i % NBUF

            @pl.when(i + NBUF - 1 < NB)
            def _():
                x_copy(i + NBUF - 1, (i + NBUF - 1) % NBUF).start()
                h_in(i + NBUF - 1, (i + NBUF - 1) % NBUF).start()

            x_copy(i, slot).wait()
            h_in(i, slot).wait()

            @pl.when(i >= NBUF)
            def _():
                o_copy(i - NBUF, slot).wait()

            for r0 in range(0, TM, M2):
                hv = h_load(i, slot, r0, M2)
                y = jnp.dot(hv, w2s[...], preferred_element_type=F32)
                obuf[slot, r0:r0 + M2, :] = (y + bias + xbuf[slot, r0:r0 + M2, :].astype(F32)).astype(BF16)
            o_copy(i, slot).start()
            return carry

        jax.lax.fori_loop(0, NB, p2, 0)
        for s in range(NBUF):
            i = NB - NBUF + s
            o_copy(i, i % NBUF).wait()

    def fn(x, dw, w1, w2, g, b):
        B, H, W, C = x.shape
        N = B * H * W
        D = w1.shape[1]
        NB = N // TM
        vm = pl.BlockSpec(memory_space=pltpu.VMEM)
        anyspec = pl.BlockSpec(memory_space=pl.ANY)
        out, _ = pl.pallas_call(
            kernel,
            in_specs=[anyspec, vm, vm, vm, vm, vm],
            out_specs=[anyspec, anyspec],
            out_shape=[jax.ShapeDtypeStruct((N, C), x.dtype), jax.ShapeDtypeStruct((NB * TH, D), BF16)],
            scratch_shapes=[
                pltpu.VMEM((NBUF, TM, C), BF16),
                pltpu.VMEM((NBUF, TH, D), BF16),
                pltpu.VMEM((NBUF, TM, C), BF16),
                pltpu.VMEM((NB, max(TC, 16), D), BF16),
                pltpu.VMEM((D, C), BF16),
                pltpu.VMEM((8, D), F32),
                pltpu.SemaphoreType.DMA((NBUF,)),
                pltpu.SemaphoreType.DMA((NBUF,)),
                pltpu.SemaphoreType.DMA((NBUF,)),
            ],
            compiler_params=pltpu.CompilerParams(vmem_limit_bytes=vmem_mb * 1024 * 1024),
        )(x.reshape(N, C), dw.reshape(1, C), w1, w2, g.reshape(1, D), b.reshape(1, D))
        return out.reshape(x.shape)

    return fn


@jax.jit
def pallas_standalone__modern_conv_block_slak__vision_kernel(x, dw, w1, w2, grn_g, grn_b):
    return make()(x, dw, w1, w2, grn_g, grn_b)
```

```python
import numpy as np
import jax
import jax.numpy as jnp
import jax.experimental.pallas as pl
import jax.experimental.pallas.tpu as pltpu

F32 = jnp.float32
BF16 = jnp.bfloat16
U32 = jnp.uint32
_C0 = float(np.sqrt(2.0 / np.pi))
ALPHA = float((_C0 * 0.044715) ** (1.0 / 3.0))
BETA = _C0 / ALPHA
HSCALE = 0.5 / ALPHA

VB = [
    (0, 0, 0, -1, 1, 0, -1, 0, 0),
    (-1, 0, 0, -1, 0, 1, 0, 0, 0),
    (0, 0, -1, 0, 0, 0, -1, 0, 1),
    (1, -1, 0, 0, 0, 0, 0, 1, 0),
    (0, 0, 0, 0, 0, -1, 0, -1, -1),
    (0, -1, -1, 0, -1, 0, 0, 0, 0),
    (0, 0, 1, 0, 0, 0, 0, 0, 0),
    (0, 0, 0, 0, 0, 0, 0, -1, 0),
    (0, 0, -1, 0, 0, 0, 0, -1, 0),
    (-1, 0, 0, 0, 0, 0, 0, 0, 0),
    (0, 0, 0, 0, 0, 0, -1, 0, 0),
    (1, 0, 0, 0, 1, 0, 0, 0, 0),
    (0, 0, 0, 0, 0, 1, 1, 0, 0),
    (0, 0, 0, 0, -1, 0, 0, 0, 0),
    (0, 0, 0, 0, 0, -1, 0, 0, 0),
]


def a_forms(a):
    a0, a1, a2, a3, a4, a5 = a
    d54 = a5 - a4
    d10 = a1 - a0
    e = a3 - d10
    f = d54 + a2
    return [a4, a1, a2, a3, a2 + a5, a0 + a3, a0 + a2, a3 + a5, a3 - a2, d10, d54, e, f, a4 - e, a1 - f]


CPROG = [
    ("t1", "p10", 1, "p12"), ("t2", "t1", -1, "p14"),
    ("u0", "t2", 1, "p9"), ("c0", "u0", -1, "p1"),
    ("u2", "t2", 1, "p2"), ("c2", "u2", 1, "p6"),
    ("t3", "p11", -1, "p9"), ("t4", "t3", -1, "p13"),
    ("u3", "t4", -1, "p10"), ("c3", "u3", -1, "p0"),
    ("u4", "t4", -1, "p3"), ("c4", "u4", -1, "p7"),
    ("u5", "p7", -1, "t1"), ("v5", "u5", -1, "p2"), ("w5", "v5", -1, "p8"), ("c5", "w5", -1, "p4"),
    ("u1", "p3", -1, "t3"), ("v1", "u1", -1, "p6"), ("w1", "v1", 1, "p8"), ("c1", "w1", -1, "p5"),
]
CDEF = {n: (l, s, r) for n, l, s, r in CPROG}


class CSide:
    def __init__(self):
        self.v = {}

    def ready(self, n):
        return n in self.v or (n in CDEF and self.ready(CDEF[n][0]) and self.ready(CDEF[n][2]))

    def get(self, n):
        if n not in self.v:
            l, s, r = CDEF[n]
            self.v[n] = self.get(l) + self.get(r) if s > 0 else self.get(l) - self.get(r)
        return self.v[n]

    def push(self, r, val):
        self.v["p%d" % r] = val
        done = []
        for n, _, _, _ in CPROG:
            if n[0] in "tc" and n not in self.v and self.ready(n):
                self.get(n)
                if n[0] == "c":
                    done.append((int(n[1]), self.v[n]))
        return done


def combine(coefs, get):
    acc = None
    for j, c in enumerate(coefs):
        if c:
            v = get(j)
            acc = (v if c > 0 else -v) if acc is None else (acc + v if c > 0 else acc - v)
    return acc


def pack(v):
    return pltpu.bitcast(v.astype(BF16), U32)


def unpack(v):
    return pltpu.bitcast(v, BF16)


ORD1 = (10, 12, 14, 9, 1, 2, 6, 11, 13, 0, 3, 7, 8, 4, 5)
ORD2 = (1, 2, 3, 0, 10, 12, 14, 9, 6, 11, 13, 7, 8, 4, 5)


def make(TM=1024, TC=256, M=64, M2=128, NBUF=2, vmem_mb=127, only=None, ord1=ORD1, ord2=ORD2,
         LQ=0, flags=None, NBC=None):
    TH = TM - TC
    NCH = TM // (2 * M)
    NX = NBUF + 1

    def kernel(x_hbm, dw_ref, w1_ref, w2_ref, g_ref, b_ref, o_hbm, h_hbm,
               xbuf, hbuf, obuf, hcache, wc1, wc2, fbuf, ssq, sem_x, sem_h, sem_o):
        N, C = x_hbm.shape
        D = w1_ref.shape[1]
        NB = N // TM
        NT = D // 128
        G = NT // 3
        GW = G * 128

        def x_copy(i):
            return pltpu.make_async_copy(x_hbm.at[pl.ds(i * TM, TM)], xbuf.at[i % NX], sem_x.at[i % NX])

        def h_out(i):
            return pltpu.make_async_copy(hbuf.at[i % NBUF], h_hbm.at[i], sem_h.at[i % NBUF])

        def h_in(i):
            return pltpu.make_async_copy(h_hbm.at[i], hbuf.at[i % NBUF], sem_h.at[i % NBUF])

        def o_copy(i):
            return pltpu.make_async_copy(obuf.at[i % NBUF], o_hbm.at[pl.ds(i * TM, TM)], sem_o.at[i % NBUF])

        def ln_half(xs, r0):
            dw = dw_ref[...].astype(F32)
            xv = xbuf[xs, pl.ds(r0, M), :].astype(F32) * dw
            mu = jnp.sum(xv, axis=-1, keepdims=True) * (1.0 / C)
            xc = xv - mu
            var = jnp.sum(xc * xc, axis=-1, keepdims=True) * (1.0 / (C * ALPHA * ALPHA))
            av = xc * jax.lax.rsqrt(var + 1e-5 / (ALPHA * ALPHA))
            return [av[:, k * 128:(k + 1) * 128] for k in range(3)]

        def ln_forms(xs, r0):
            return [f.astype(BF16) for f in a_forms(ln_half(xs, r0) + ln_half(xs, r0 + M))]

        def p1(i, carry):
            @pl.when(i + NX - 1 < NB)
            def _():
                x_copy(i + NX - 1).start()

            @pl.when(i + 1 < NB)
            def _():
                x_copy(i + 1).wait()

            @pl.when(i >= NBUF)
            def _():
                h_out(i - NBUF).wait()

            acc = [None] * NT
            nf = [fbuf[r] for r in range(15)]
            for ch in range(NCH):
                ref, bi, r0 = (hcache, i, ch * 2 * M - TH) if ch * 2 * M >= TH else (hbuf, i % NBUF, ch * 2 * M)
                nxt = (i % NX, (ch + 1) * 2 * M) if ch < NCH - 1 else (jnp.minimum(i + 1, NB - 1) % NX, 0)
                cur = nf
                for q in range(G):
                    if q == LQ:
                        nf = ln_forms(*nxt)
                    cs = CSide()
                    for r in ord1:
                        p = jnp.dot(cur[r], unpack(wc1[r, q]), preferred_element_type=F32)
                        for c, y in cs.push(r, p):
                            t = jnp.tanh(y * (y * y + BETA))
                            hv = y + y * t
                            sq = hv * hv
                            n = (c % 3) * G + q
                            for k in range(M // 8):
                                u = sq[8 * k:8 * k + 8]
                                acc[n] = u if acc[n] is None else acc[n] + u
                            ref[bi, n, pl.ds(r0 + (c // 3) * M, M), :] = hv.astype(BF16)
            for r in range(15):
                fbuf[r] = nf[r]
            for n in range(NT):
                ssq[:, n * 128:(n + 1) * 128] += acc[n]
            h_out(i).start()
            return carry

        if only != 2:
            for s in range(NX - 1):
                x_copy(s).start()
            ssq[...] = jnp.zeros_like(ssq)
            for r in range(15):
                for t in range(G):
                    get = lambda j: w1_ref[(j // 3) * 128:(j // 3 + 1) * 128,
                                           ((j % 3) * G + t) * 128:((j % 3) * G + t + 1) * 128].astype(F32)
                    wc1[r, t] = pack(combine(VB[r], get))
            x_copy(0).wait()
            for r, f in enumerate(ln_forms(0, 0)):
                fbuf[r] = f
            jax.lax.fori_loop(0, NB, p1, 0)
            for s in range(NBUF):
                h_out(NB - NBUF + s).wait()
        if only == 1:
            return

        for s in range(NBUF - 1):
            x_copy(s).start()
            h_in(s).start()

        gx = jnp.sqrt(jnp.sum(ssq[...], axis=0, keepdims=True) * (HSCALE * HSCALE) + 1e-6)
        nx = gx / (jnp.mean(gx, axis=-1, keepdims=True) + 1e-6)
        sc = (1.0 + g_ref[...].astype(F32) * nx) * HSCALE
        scT = jnp.broadcast_to(sc, (128, D)).T
        get = lambda j: (w2_ref[(j // 3) * GW:(j // 3 + 1) * GW, (j % 3) * 128:(j % 3 + 1) * 128].astype(F32)
                         * scT[(j // 3) * GW:(j // 3 + 1) * GW])
        for r in range(15):
            wc2[r] = pack(combine(VB[r], get))
        bias = jnp.dot(jnp.broadcast_to(b_ref[...], (16, D)), w2_ref[...], preferred_element_type=F32)[0:1]

        def p2(i, carry):
            @pl.when(i + NBUF - 1 < NB)
            def _():
                x_copy(i + NBUF - 1).start()
                h_in(i + NBUF - 1).start()

            x_copy(i).wait()
            h_in(i).wait()

            @pl.when(i >= NBUF)
            def _():
                o_copy(i - NBUF).wait()

            for ch in range(TM // (2 * M2)):
                ref, r0 = (hcache.at[i], ch * 2 * M2 - TH) if ch * 2 * M2 >= TH else (hbuf.at[i % NBUF], ch * 2 * M2)
                raw = [jnp.concatenate([ref[k * G + q, pl.ds(r0 + hf * M2, M2), :] for q in range(G)], axis=1)
                       for hf in range(2) for k in range(3)]
                forms = a_forms([v.astype(F32) for v in raw])
                forms = [raw[4], raw[1], raw[2], raw[3]] + [f.astype(BF16) for f in forms[4:]]
                cs = CSide()
                for r in ord2:
                    p = jnp.dot(forms[r], unpack(wc2[r]), preferred_element_type=F32)
                    for c, y in cs.push(r, p):
                        rs = pl.ds(ch * 2 * M2 + (c // 3) * M2, M2)
                        cl = slice((c % 3) * 128, (c % 3 + 1) * 128)
                        obuf[i % NBUF, rs, cl] = (y + bias[:, cl] + xbuf[i % NX, rs, cl].astype(F32)).astype(BF16)
            o_copy(i).start()
            return carry

        jax.lax.fori_loop(0, NB, p2, 0)
        for s in range(NBUF):
            o_copy(NB - NBUF + s).wait()

    def fn(x, dw, w1, w2, g, b):
        B, H, W, C = x.shape
        N = B * H * W
        D = w1.shape[1]
        NB = N // TM
        NT = D // 128
        vm = pl.BlockSpec(memory_space=pltpu.VMEM)
        anyspec = pl.BlockSpec(memory_space=pl.ANY)
        out, _ = pl.pallas_call(
            kernel,
            in_specs=[anyspec, vm, vm, vm, vm, vm],
            out_specs=[anyspec, anyspec],
            out_shape=[jax.ShapeDtypeStruct((N, C), x.dtype), jax.ShapeDtypeStruct((NB, NT, TH, 128), BF16)],
            scratch_shapes=[
                pltpu.VMEM((NX, TM, C), BF16),
                pltpu.VMEM((NBUF, NT, TH, 128), BF16),
                pltpu.VMEM((NBUF, TM, C), BF16),
                pltpu.VMEM((NBC or NB, NT, TC, 128), BF16),
                pltpu.VMEM((15, NT // 3, 64, 128), U32),
                pltpu.VMEM((15, D // 6, 128), U32),
                pltpu.VMEM((15, M, 128), BF16),
                pltpu.VMEM((8, D), F32),
                pltpu.SemaphoreType.DMA((NX,)),
                pltpu.SemaphoreType.DMA((NBUF,)),
                pltpu.SemaphoreType.DMA((NBUF,)),
            ],
            compiler_params=pltpu.CompilerParams(vmem_limit_bytes=vmem_mb * 1024 * 1024, flags=flags),
        )(x.reshape(N, C), dw.reshape(1, C), w1, w2, g.reshape(1, D), b.reshape(1, D))
        return out.reshape(x.shape)

    return fn


@jax.jit
def pallas_standalone__modern_conv_block_slak__vision_kernel(x, dw, w1, w2, grn_g, grn_b):
    return make()(x, dw, w1, w2, grn_g, grn_b)
```

```python
import numpy as np
import jax
import jax.numpy as jnp
import jax.experimental.pallas as pl
import jax.experimental.pallas.tpu as pltpu

F32 = jnp.float32
BF16 = jnp.bfloat16
U32 = jnp.uint32
_C0 = float(np.sqrt(2.0 / np.pi))
ALPHA = float((_C0 * 0.044715) ** (1.0 / 3.0))
BETA = _C0 / ALPHA
HSCALE = 0.5 / ALPHA

VB = [
    (0, 0, 0, -1, 1, 0, -1, 0, 0),
    (-1, 0, 0, -1, 0, 1, 0, 0, 0),
    (0, 0, -1, 0, 0, 0, -1, 0, 1),
    (1, -1, 0, 0, 0, 0, 0, 1, 0),
    (0, 0, 0, 0, 0, -1, 0, -1, -1),
    (0, -1, -1, 0, -1, 0, 0, 0, 0),
    (0, 0, 1, 0, 0, 0, 0, 0, 0),
    (0, 0, 0, 0, 0, 0, 0, -1, 0),
    (0, 0, -1, 0, 0, 0, 0, -1, 0),
    (-1, 0, 0, 0, 0, 0, 0, 0, 0),
    (0, 0, 0, 0, 0, 0, -1, 0, 0),
    (1, 0, 0, 0, 1, 0, 0, 0, 0),
    (0, 0, 0, 0, 0, 1, 1, 0, 0),
    (0, 0, 0, 0, -1, 0, 0, 0, 0),
    (0, 0, 0, 0, 0, -1, 0, 0, 0),
]


def a_forms(a):
    a0, a1, a2, a3, a4, a5 = a
    d54 = a5 - a4
    d10 = a1 - a0
    e = a3 - d10
    f = d54 + a2
    return [a4, a1, a2, a3, a2 + a5, a0 + a3, a0 + a2, a3 + a5, a3 - a2, d10, d54, e, f, a4 - e, a1 - f]


CPROG = [
    ("t1", "p10", 1, "p12"), ("t2", "t1", -1, "p14"),
    ("u0", "t2", 1, "p9"), ("c0", "u0", -1, "p1"),
    ("u2", "t2", 1, "p2"), ("c2", "u2", 1, "p6"),
    ("t3", "p11", -1, "p9"), ("t4", "t3", -1, "p13"),
    ("u3", "t4", -1, "p10"), ("c3", "u3", -1, "p0"),
    ("u4", "t4", -1, "p3"), ("c4", "u4", -1, "p7"),
    ("u5", "p7", -1, "t1"), ("v5", "u5", -1, "p2"), ("w5", "v5", -1, "p8"), ("c5", "w5", -1, "p4"),
    ("u1", "p3", -1, "t3"), ("v1", "u1", -1, "p6"), ("w1", "v1", 1, "p8"), ("c1", "w1", -1, "p5"),
]
CDEF = {n: (l, s, r) for n, l, s, r in CPROG}


class CSide:
    def __init__(self):
        self.v = {}

    def ready(self, n):
        return n in self.v or (n in CDEF and self.ready(CDEF[n][0]) and self.ready(CDEF[n][2]))

    def get(self, n):
        if n not in self.v:
            l, s, r = CDEF[n]
            self.v[n] = self.get(l) + self.get(r) if s > 0 else self.get(l) - self.get(r)
        return self.v[n]

    def push(self, r, val):
        self.v["p%d" % r] = val
        done = []
        for n, _, _, _ in CPROG:
            if n[0] in "tc" and n not in self.v and self.ready(n):
                self.get(n)
                if n[0] == "c":
                    done.append((int(n[1]), self.v[n]))
        return done


def combine(coefs, get):
    acc = None
    for j, c in enumerate(coefs):
        if c:
            v = get(j)
            acc = (v if c > 0 else -v) if acc is None else (acc + v if c > 0 else acc - v)
    return acc


def pack(v):
    return pltpu.bitcast(v.astype(BF16), U32)


def unpack(v):
    return pltpu.bitcast(v, BF16)


ORD1 = (10, 12, 14, 9, 1, 2, 6, 11, 13, 0, 3, 7, 8, 4, 5)
ORD2 = (1, 2, 3, 0, 10, 12, 14, 9, 6, 11, 13, 7, 8, 4, 5)


def make(TM=1024, TC=256, M=64, M2=128, NBUF=3, NX=3, NO=2, vmem_mb=128, only=None, ord1=ORD1, ord2=ORD2,
         LQ=0, flags=None, NBC=None):
    TH = TM - TC
    NCH = TM // (2 * M)

    def kernel(x_hbm, dw_ref, w1_ref, w2_ref, g_ref, b_ref, o_hbm, h_hbm,
               xbuf, hbuf, obuf, hcache, wc1, wc2, fbuf, ssq, sem_x, sem_h, sem_o):
        N, C = x_hbm.shape
        D = w1_ref.shape[1]
        NB = N // TM
        NT = D // 128
        G = NT // 3
        GW = G * 128

        def x_copy(i):
            return pltpu.make_async_copy(x_hbm.at[pl.ds(i * TM, TM)], xbuf.at[i % NX], sem_x.at[i % NX])

        def h_out(i):
            return pltpu.make_async_copy(hbuf.at[i % NBUF], h_hbm.at[i - NBUF], sem_h.at[i % NBUF])

        def h_in(i):
            return pltpu.make_async_copy(h_hbm.at[i - NBUF], hbuf.at[i % NBUF], sem_h.at[i % NBUF])

        def o_copy(i):
            return pltpu.make_async_copy(obuf.at[i % NO], o_hbm.at[pl.ds(i * TM, TM)], sem_o.at[i % NO])

        def ln_half(xs, r0):
            dw = dw_ref[...].astype(F32)
            xv = xbuf[xs, pl.ds(r0, M), :].astype(F32) * dw
            mu = jnp.sum(xv, axis=-1, keepdims=True) * (1.0 / C)
            xc = xv - mu
            var = jnp.sum(xc * xc, axis=-1, keepdims=True) * (1.0 / (C * ALPHA * ALPHA))
            av = xc * jax.lax.rsqrt(var + 1e-5 / (ALPHA * ALPHA))
            return [av[:, k * 128:(k + 1) * 128] for k in range(3)]

        def ln_forms(xs, r0):
            return [f.astype(BF16) for f in a_forms(ln_half(xs, r0) + ln_half(xs, r0 + M))]

        def p1(step, carry):
            i = NB - 1 - step

            @pl.when(i - (NX - 1) >= 0)
            def _():
                x_copy(i - (NX - 1)).start()

            @pl.when(i >= 1)
            def _():
                x_copy(i - 1).wait()

            @pl.when(i + NBUF < NB)
            def _():
                h_out(i + NBUF).wait()

            acc = [None] * NT
            nf = [fbuf[r] for r in range(15)]
            for ch in range(NCH):
                ref, bi, r0 = (hcache, i, ch * 2 * M - TH) if ch * 2 * M >= TH else (hbuf, i % NBUF, ch * 2 * M)
                nxt = (i % NX, (ch + 1) * 2 * M) if ch < NCH - 1 else (jnp.maximum(i - 1, 0) % NX, 0)
                cur = nf
                for q in range(G):
                    if q == LQ:
                        nf = ln_forms(*nxt)
                    cs = CSide()
                    for r in ord1:
                        p = jnp.dot(cur[r], unpack(wc1[r, q]), preferred_element_type=F32)
                        for c, y in cs.push(r, p):
                            t = jnp.tanh(y * (y * y + BETA))
                            hv = y + y * t
                            sq = hv * hv
                            n = (c % 3) * G + q
                            for k in range(M // 8):
                                u = sq[8 * k:8 * k + 8]
                                acc[n] = u if acc[n] is None else acc[n] + u
                            ref[bi, n, pl.ds(r0 + (c // 3) * M, M), :] = hv.astype(BF16)
            for r in range(15):
                fbuf[r] = nf[r]
            for n in range(NT):
                ssq[:, n * 128:(n + 1) * 128] += acc[n]

            @pl.when(i >= NBUF)
            def _():
                h_out(i).start()

            return carry

        if only != 2:
            for s in range(NX - 1):
                x_copy(NB - 1 - s).start()
            ssq[...] = jnp.zeros_like(ssq)
            for r in range(15):
                for t in range(G):
                    get = lambda j: w1_ref[(j // 3) * 128:(j // 3 + 1) * 128,
                                           ((j % 3) * G + t) * 128:((j % 3) * G + t + 1) * 128].astype(F32)
                    wc1[r, t] = pack(combine(VB[r], get))
            x_copy(NB - 1).wait()
            for r, f in enumerate(ln_forms((NB - 1) % NX, 0)):
                fbuf[r] = f
            jax.lax.fori_loop(0, NB, p1, 0)
        if only == 1:
            return

        if only == 2:
            for s in range(NX):
                x_copy(s).start()
                x_copy(s).wait()

        gx = jnp.sqrt(jnp.sum(ssq[...], axis=0, keepdims=True) * (HSCALE * HSCALE) + 1e-6)
        nx = gx / (jnp.mean(gx, axis=-1, keepdims=True) + 1e-6)
        sc = (1.0 + g_ref[...].astype(F32) * nx) * HSCALE
        scT = jnp.broadcast_to(sc, (128, D)).T
        get = lambda j: (w2_ref[(j // 3) * GW:(j // 3 + 1) * GW, (j % 3) * 128:(j % 3 + 1) * 128].astype(F32)
                         * scT[(j // 3) * GW:(j // 3 + 1) * GW])
        for r in range(15):
            wc2[r] = pack(combine(VB[r], get))
        bias = jnp.dot(jnp.broadcast_to(b_ref[...], (16, D)), w2_ref[...], preferred_element_type=F32)[0:1]

        def p2(i, carry):
            @pl.when(jnp.logical_and(i >= 1, i + NBUF - 1 < NB))
            def _():
                h_in(i + NBUF - 1).start()

            @pl.when(jnp.logical_and(i >= 1, i + NX - 1 < NB))
            def _():
                x_copy(i + NX - 1).start()

            @pl.when(i >= NX)
            def _():
                x_copy(i).wait()

            @pl.when(i >= NBUF)
            def _():
                h_in(i).wait()

            @pl.when(i >= NO)
            def _():
                o_copy(i - NO).wait()

            for ch in range(TM // (2 * M2)):
                ref, r0 = (hcache.at[i], ch * 2 * M2 - TH) if ch * 2 * M2 >= TH else (hbuf.at[i % NBUF], ch * 2 * M2)
                raw = [jnp.concatenate([ref[k * G + q, pl.ds(r0 + hf * M2, M2), :] for q in range(G)], axis=1)
                       for hf in range(2) for k in range(3)]
                forms = a_forms([v.astype(F32) for v in raw])
                forms = [raw[4], raw[1], raw[2], raw[3]] + [f.astype(BF16) for f in forms[4:]]
                cs = CSide()
                for r in ord2:
                    p = jnp.dot(forms[r], unpack(wc2[r]), preferred_element_type=F32)
                    for c, y in cs.push(r, p):
                        rs = pl.ds(ch * 2 * M2 + (c // 3) * M2, M2)
                        cl = slice((c % 3) * 128, (c % 3 + 1) * 128)
                        obuf[i % NO, rs, cl] = (y + bias[:, cl] + xbuf[i % NX, rs, cl].astype(F32)).astype(BF16)
            o_copy(i).start()
            return carry

        jax.lax.fori_loop(0, NB, p2, 0)
        for s in range(NO):
            o_copy(NB - NO + s).wait()

    def fn(x, dw, w1, w2, g, b):
        B, H, W, C = x.shape
        N = B * H * W
        D = w1.shape[1]
        NB = N // TM
        NT = D // 128
        vm = pl.BlockSpec(memory_space=pltpu.VMEM)
        anyspec = pl.BlockSpec(memory_space=pl.ANY)
        out, _ = pl.pallas_call(
            kernel,
            in_specs=[anyspec, vm, vm, vm, vm, vm],
            out_specs=[anyspec, anyspec],
            out_shape=[jax.ShapeDtypeStruct((N, C), x.dtype), jax.ShapeDtypeStruct((NB - NBUF, NT, TH, 128), BF16)],
            scratch_shapes=[
                pltpu.VMEM((NX, TM, C), BF16),
                pltpu.VMEM((NBUF, NT, TH, 128), BF16),
                pltpu.VMEM((NO, TM, C), BF16),
                pltpu.VMEM((NBC or NB, NT, TC, 128), BF16),
                pltpu.VMEM((15, NT // 3, 64, 128), U32),
                pltpu.VMEM((15, D // 6, 128), U32),
                pltpu.VMEM((15, M, 128), BF16),
                pltpu.VMEM((8, D), F32),
                pltpu.SemaphoreType.DMA((NX,)),
                pltpu.SemaphoreType.DMA((NBUF,)),
                pltpu.SemaphoreType.DMA((NO,)),
            ],
            compiler_params=pltpu.CompilerParams(vmem_limit_bytes=vmem_mb * 1024 * 1024, flags=flags),
        )(x.reshape(N, C), dw.reshape(1, C), w1, w2, g.reshape(1, D), b.reshape(1, D))
        return out.reshape(x.shape)

    return fn


@jax.jit
def pallas_standalone__modern_conv_block_slak__vision_kernel(x, dw, w1, w2, grn_g, grn_b):
    return make()(x, dw, w1, w2, grn_g, grn_b)
```

```python
import numpy as np
import jax
import jax.numpy as jnp
import jax.experimental.pallas as pl
import jax.experimental.pallas.tpu as pltpu

F32 = jnp.float32
BF16 = jnp.bfloat16
U32 = jnp.uint32

_C0 = float(np.sqrt(2.0 / np.pi))
ALPHA = float((_C0 * 0.044715) ** (1.0 / 3.0))
BETA = _C0 / ALPHA
HSCALE = 0.5 / ALPHA

B_FORMS = (
    (0, 0, 0, -1, 1, 0, -1, 0, 0),
    (-1, 0, 0, -1, 0, 1, 0, 0, 0),
    (0, 0, -1, 0, 0, 0, -1, 0, 1),
    (1, -1, 0, 0, 0, 0, 0, 1, 0),
    (0, 0, 0, 0, 0, -1, 0, -1, -1),
    (0, -1, -1, 0, -1, 0, 0, 0, 0),
    (0, 0, 1, 0, 0, 0, 0, 0, 0),
    (0, 0, 0, 0, 0, 0, 0, -1, 0),
    (0, 0, -1, 0, 0, 0, 0, -1, 0),
    (-1, 0, 0, 0, 0, 0, 0, 0, 0),
    (0, 0, 0, 0, 0, 0, -1, 0, 0),
    (1, 0, 0, 0, 1, 0, 0, 0, 0),
    (0, 0, 0, 0, 0, 1, 1, 0, 0),
    (0, 0, 0, 0, -1, 0, 0, 0, 0),
    (0, 0, 0, 0, 0, -1, 0, 0, 0),
)


def a_forms(a):
    a0, a1, a2, a3, a4, a5 = a
    d54 = a5 - a4
    d10 = a1 - a0
    e = a3 - d10
    f = d54 + a2
    return [a4, a1, a2, a3, a2 + a5, a0 + a3, a0 + a2, a3 + a5, a3 - a2, d10, d54, e, f, a4 - e, a1 - f]


C_SUMS = {
    "t1": {"p10": 1, "p12": 1},
    "t2": {"t1": 1, "p14": -1},
    "t3": {"p11": 1, "p9": -1},
    "t4": {"t3": 1, "p13": -1},
    "c0": {"t2": 1, "p9": 1, "p1": -1},
    "c1": {"p3": 1, "t3": -1, "p6": -1, "p8": 1, "p5": -1},
    "c2": {"t2": 1, "p2": 1, "p6": 1},
    "c3": {"t4": 1, "p10": -1, "p0": -1},
    "c4": {"t4": 1, "p3": -1, "p7": -1},
    "c5": {"p7": 1, "t1": -1, "p2": -1, "p8": -1, "p4": -1},
}


def block_products(order, product):
    partial = {name: None for name in C_SUMS}
    missing = {name: len(terms) for name, terms in C_SUMS.items()}
    for r in order:
        arrived = [("p%d" % r, product(r))]
        while arrived:
            term, v = arrived.pop(0)
            for name, terms in C_SUMS.items():
                if term not in terms:
                    continue
                sign = terms[term]
                if partial[name] is None:
                    partial[name] = (sign, v)
                else:
                    s0, v0 = partial[name]
                    partial[name] = (s0, v0 + v) if s0 == sign else (1, v0 - v if s0 > 0 else v - v0)
                missing[name] -= 1
                if missing[name] == 0:
                    assert partial[name][0] > 0
                    if name[0] == "t":
                        arrived.append((name, partial[name][1]))
                    else:
                        yield int(name[1]), partial[name][1]


def signed_sum(coefs, get):
    acc = None
    for j, c in enumerate(coefs):
        if c:
            v = get(j)
            acc = (v if c > 0 else -v) if acc is None else (acc + v if c > 0 else acc - v)
    return acc


ORDER1 = (10, 12, 14, 9, 1, 2, 6, 11, 13, 0, 3, 7, 8, 4, 5)
ORDER2 = (1, 2, 3, 0, 10, 12, 14, 9, 6, 11, 13, 7, 8, 4, 5)


def make(TM=1536, TC=384, US=16, NL=3, M2=32, NH=3, NX=4, ND=3,  ord1=ORDER1, ord2=ORDER2,
         only=None, flags=None, nobc=True, nodma=False):
    TH = TM - TC

    def kernel(x_hbm, dw_ref, w1_hbm, w2_ref, g_ref, b_ref, o_hbm, h_hbm,
               xbuf, hbuf, hcache, wc, fbuf, ybuf, ssq, sem_x, sem_h, sem_w):
        N, C = x_hbm.shape
        D = w1_hbm.shape[1]
        NB = N // TM
        NT = D // 128
        G = NT // 3

        def x_in(i):
            return pltpu.make_async_copy(x_hbm.at[pl.ds(i * TM, TM)], xbuf.at[i % NX], sem_x.at[i % NX])

        def o_out(i):
            return pltpu.make_async_copy(xbuf.at[i % NX], o_hbm.at[pl.ds(i * TM, TM)], sem_x.at[i % NX])

        def h_out(i):
            return pltpu.make_async_copy(hbuf.at[i % NH], h_hbm.at[i - NH], sem_h.at[i % NH])

        def h_in(i):
            return pltpu.make_async_copy(h_hbm.at[i - NH], hbuf.at[i % NH], sem_h.at[i % NH])

        def h_place(i, r0):
            return (hcache, i, r0 - TH) if r0 >= TH else (hbuf, i % NH, r0)

        def weight(r, q):
            return pltpu.bitcast(wc[r, q], BF16)

        def layernorm(slot, starts):
            dw = dw_ref[...].astype(F32)
            xc, ss = [], []
            for r0 in starts:
                xv = xbuf[slot, pl.ds(r0, 8), :].astype(F32) * dw
                xc.append(xv - jnp.sum(xv, axis=-1, keepdims=True) * (1.0 / C))
                ss.append(jnp.sum(xc[-1] * xc[-1], axis=-1, keepdims=True))
            inv_std = lambda v: jax.lax.rsqrt(v * (1.0 / (C * ALPHA * ALPHA)) + 1e-5 / (ALPHA * ALPHA))
            return [v * inv_std(t) for v, t in zip(xc, ss)]

        def left_unit(slot, u):
            groups = range(0, US, 8)
            a = layernorm(slot, [(2 * u + half) * US + k for k in groups for half in range(2)])
            forms = [a_forms([v[:, k * 128:(k + 1) * 128] for v in a[2 * g:2 * g + 2] for k in range(3)])
                     for g in range(len(groups))]
            return [jnp.concatenate([f[r] for f in forms], axis=0) for r in range(15)]

        def activate(y, places, c, q, acc):
            n = (c % 3) * G + q
            h = y + y * jnp.tanh(y * (y * y + BETA))
            sq = h * h
            for k in range(0, y.shape[0], 8):
                acc[n] = sq[k:k + 8] if acc[n] is None else acc[n] + sq[k:k + 8]
            hb = h.astype(BF16)
            for k, (i, u) in enumerate(places):
                ref, j, r = h_place(i, (2 * u + c // 3) * US)
                ref[j, n, pl.ds(r, US), :] = hb[k * US:(k + 1) * US]

        def flush(acc):
            for n, v in enumerate(acc):
                if v is not None:
                    ssq[:, n * 128:(n + 1) * 128] += v

        def first_matmul(units, q):
            def product(r):
                fresh = [u[r] for u in units if u[r].dtype == F32]
                lhs = [u[r] for u in units if u[r].dtype == BF16]
                if fresh:
                    lhs.append(jnp.concatenate(fresh, axis=0).astype(BF16))
                return jnp.dot(jnp.concatenate(lhs, axis=0), weight(r, q), preferred_element_type=F32)
            return block_products(ord1, product)

        NU = TM // (2 * US)
        NS = NU * G // NL
        live_at = lambda t: [u for u in range(1 - NL, NU) if 0 <= t - (G * u) // NL < G]
        done_order = [c for c, _ in block_products(ord1, lambda r: 0.0)]
        deferred = done_order[6 - ND:] if ND else []

        def activate_deferred(i, acc):
            for k, c in enumerate(deferred):
                activate(ybuf[k], [(i, u) for u in live_at(NS - 1)], c, (NS - 1) % G, acc)

        def pass1(step, carry):
            i = NB - 1 - step

            @pl.when(i >= NX - 1)
            def _():
                x_in(i - (NX - 1)).start()

            @pl.when(i >= 1)
            def _():
                x_in(i - 1).wait()

            @pl.when(i + NH < (0 if nodma else NB))
            def _():
                h_out(i + NH).wait()

            acc = [None] * NT
            prev = jnp.minimum(i + 1, NB - 1)
            activate_deferred(prev, acc)
            units = {k - (NL - 1): [fbuf[k, r] for r in range(15)] for k in range(NL)}
            for t in range(NS):
                for u in (live_at(t + 1) if t + 1 < NS else [NU]):
                    if u not in units:
                        units[u] = left_unit(i % NX, u) if u < NU else left_unit(jnp.maximum(i - 1, 0) % NX, 0)
                live = live_at(t)
                for c, y in first_matmul([units[u] for u in live], t % G):
                    if t == NS - 1 and c in deferred:
                        ybuf[deferred.index(c)] = y
                    else:
                        activate(y, [(i, u) if u >= 0 else (prev, u + NU) for u in live], c, t % G, acc)
            for k in range(NL):
                for r in range(15):
                    fbuf[k, r] = units[NU - (NL - 1) + k][r].astype(BF16)
            flush(acc)

            @pl.when(i >= (NB if nodma else NH))
            def _():
                h_out(i).start()

            return carry

        if only != 2:
            w1_in = [pltpu.make_async_copy(w1_hbm.at[pl.ds(k * 128, 128), pl.ds(n * 128, 128)],
                                           hcache.at[k, n, pl.ds(0, 128)], sem_w)
                     for k in range(3) for n in range(NT)]
            for cp in w1_in:
                cp.start()
            x_in(NB - 1).start()
            ssq[...] = jnp.zeros_like(ssq)
            ybuf[...] = jnp.zeros_like(ybuf)
            fbuf[...] = jnp.zeros_like(fbuf)
            for cp in w1_in:
                cp.wait()
            for q in range(G):
                w1_block = lambda j: hcache[j // 3, (j % 3) * G + q, pl.ds(0, 128), :].astype(F32)
                for r in range(15):
                    wc[r, q] = pltpu.bitcast(signed_sum(B_FORMS[r], w1_block).astype(BF16), U32)
            x_in(NB - 1).wait()
            for s in range(1, NX - 1):
                x_in(NB - 1 - s).start()
            for r, f in enumerate(left_unit((NB - 1) % NX, 0)):
                fbuf[NL - 1, r] = f.astype(BF16)
            jax.lax.fori_loop(0, NB, pass1, 0)
            acc = [None] * NT
            activate_deferred(0, acc)
            for t in range(G - 1):
                live = [u for u in live_at(t) if u < 0]
                if live:
                    for c, y in first_matmul([[fbuf[u + NL - 1, r] for r in range(15)] for u in live], t):
                        activate(y, [(0, NU + u) for u in live], c, t, acc)
            flush(acc)
        if only == 1:
            return
        if only == 2:
            for s in range(NX):
                x_in(s).start()
                x_in(s).wait()

        gx = jnp.sqrt(jnp.sum(ssq[...], axis=0, keepdims=True) * (HSCALE * HSCALE) + 1e-6)
        nx = gx / (jnp.mean(gx, axis=-1, keepdims=True) + 1e-6)
        scale = (1.0 + g_ref[...].astype(F32).reshape(1, D) * nx) * HSCALE
        b_row = b_ref[...].astype(F32).reshape(1, D)
        bias = jnp.dot(jnp.broadcast_to(b_row, (16, D)).astype(BF16), w2_ref[...], preferred_element_type=F32)[0:1]
        for q in range(G):
            col = [jnp.broadcast_to(scale[:, (k * G + q) * 128:(k * G + q + 1) * 128], (128, 128)).T for k in range(3)]
            blocks = [w2_ref[pl.ds(((j // 3) * G + q) * 128, 128), pl.ds((j % 3) * 128, 128)].astype(F32) * col[j // 3]
                      for j in range(9)]
            for r in range(15):
                wc[r, q] = pltpu.bitcast(signed_sum(B_FORMS[r], blocks.__getitem__).astype(BF16), U32)

        def pass2(i, carry):
            @pl.when(i >= 2)
            def _():
                o_out(i - 2).wait()

            @pl.when(jnp.logical_and(i >= 2, i + NX - 2 < NB))
            def _():
                x_in(i + NX - 2).start()

            @pl.when(jnp.logical_and(i >= 1, i + NH - 1 < NB))
            def _():
                h_in(i + NH - 1).start()

            @pl.when(i >= NH)
            def _():
                h_in(i).wait()

            @pl.when(i >= NX)
            def _():
                x_in(i).wait()

            for r0 in range(0, TM, 2 * M2):
                raw = []
                for half in range(2):
                    ref, j, r = h_place(i, r0 + half * M2)
                    raw += [jnp.concatenate([ref[j, k * G + q, pl.ds(r, M2), :] for q in range(G)], axis=1)
                            for k in range(3)]
                forms = a_forms([v.astype(F32) for v in raw])
                forms = [raw[4], raw[1], raw[2], raw[3]] + [f.astype(BF16) for f in forms[4:]]
                product = lambda r: jnp.dot(
                    forms[r], jnp.concatenate([weight(r, q) for q in range(G)], axis=0), preferred_element_type=F32)
                for c, y in block_products(ord2, product):
                    rows = pl.ds(r0 + (c // 3) * M2, M2)
                    cols = slice((c % 3) * 128, (c % 3 + 1) * 128)
                    xbuf[i % NX, rows, cols] = (y + bias[:, cols] + xbuf[i % NX, rows, cols].astype(F32)).astype(BF16)
            o_out(i).start()
            return carry

        jax.lax.fori_loop(0, NB, pass2, 0)
        o_out(NB - 2).wait()
        o_out(NB - 1).wait()

    def fn(x, dw, w1, w2, grn_g, grn_b):
        B, H, W, C = x.shape
        N = B * H * W
        D = w1.shape[1]
        NB = N // TM
        NT = D // 128
        assert (TM // (2 * US) * (NT // 3)) % NL == 0
        assert B == 1 and dw.shape[:2] == (1, 1) and C == 384 and D % 384 == 0 and N % TM == 0
        vmem = pl.BlockSpec(memory_space=pltpu.VMEM)
        hbm = pl.BlockSpec(memory_space=pl.ANY)
        out, _ = pl.pallas_call(
            kernel,
            in_specs=[hbm, vmem, hbm, vmem, vmem, vmem],
            out_specs=[hbm, hbm],
            out_shape=[jax.ShapeDtypeStruct((N, C), x.dtype), jax.ShapeDtypeStruct((NB - NH, NT, TH, 128), BF16)],
            scratch_shapes=[
                pltpu.VMEM((NX, TM, C), BF16),
                pltpu.VMEM((NH, NT, TH, 128), BF16),
                pltpu.VMEM((NB, NT, TC, 128), BF16),
                pltpu.VMEM((15, NT // 3, 64, 128), U32),
                pltpu.VMEM((NL, 15, US, 128), BF16),
                pltpu.VMEM((max(ND, 1), NL * US, 128), F32),
                pltpu.VMEM((8, D), F32),
                pltpu.SemaphoreType.DMA((NX,)),
                pltpu.SemaphoreType.DMA((NH,)),
                pltpu.SemaphoreType.DMA(()),
            ],
            compiler_params=pltpu.CompilerParams(
                vmem_limit_bytes=128 * 1024 * 1024, flags=flags, disable_bounds_checks=nobc),
        )(x.reshape(N, C), dw.reshape(1, C), w1, w2, grn_g, grn_b)
        return out.reshape(x.shape)

    return fn


@jax.jit
def pallas_standalone__modern_conv_block_slak__vision_kernel(x, dw, w1, w2, grn_g, grn_b):
    return make()(x, dw, w1, w2, grn_g, grn_b)
```

```python
import numpy as np
import jax
import jax.numpy as jnp
import jax.experimental.pallas as pl
import jax.experimental.pallas.tpu as pltpu

F32 = jnp.float32
BF16 = jnp.bfloat16
U32 = jnp.uint32

_C0 = float(np.sqrt(2.0 / np.pi))
ALPHA = float((_C0 * 0.044715) ** (1.0 / 3.0))
BETA = _C0 / ALPHA
HSCALE = 0.5 / ALPHA

B_FORMS = (
    (0, 0, 0, -1, 1, 0, -1, 0, 0),
    (-1, 0, 0, -1, 0, 1, 0, 0, 0),
    (0, 0, -1, 0, 0, 0, -1, 0, 1),
    (1, -1, 0, 0, 0, 0, 0, 1, 0),
    (0, 0, 0, 0, 0, -1, 0, -1, -1),
    (0, -1, -1, 0, -1, 0, 0, 0, 0),
    (0, 0, 1, 0, 0, 0, 0, 0, 0),
    (0, 0, 0, 0, 0, 0, 0, -1, 0),
    (0, 0, -1, 0, 0, 0, 0, -1, 0),
    (-1, 0, 0, 0, 0, 0, 0, 0, 0),
    (0, 0, 0, 0, 0, 0, -1, 0, 0),
    (1, 0, 0, 0, 1, 0, 0, 0, 0),
    (0, 0, 0, 0, 0, 1, 1, 0, 0),
    (0, 0, 0, 0, -1, 0, 0, 0, 0),
    (0, 0, 0, 0, 0, -1, 0, 0, 0),
)


def a_forms(a):
    a0, a1, a2, a3, a4, a5 = a
    d54 = a5 - a4
    d10 = a1 - a0
    e = a3 - d10
    f = d54 + a2
    return [a4, a1, a2, a3, a2 + a5, a0 + a3, a0 + a2, a3 + a5, a3 - a2, d10, d54, e, f, a4 - e, a1 - f]


C_SUMS = {
    "t1": {"p10": 1, "p12": 1},
    "t2": {"t1": 1, "p14": -1},
    "t3": {"p11": 1, "p9": -1},
    "t4": {"t3": 1, "p13": -1},
    "c0": {"t2": 1, "p9": 1, "p1": -1},
    "c1": {"p3": 1, "t3": -1, "p6": -1, "p8": 1, "p5": -1},
    "c2": {"t2": 1, "p2": 1, "p6": 1},
    "c3": {"t4": 1, "p10": -1, "p0": -1},
    "c4": {"t4": 1, "p3": -1, "p7": -1},
    "c5": {"p7": 1, "t1": -1, "p2": -1, "p8": -1, "p4": -1},
}


def block_products(order, product):
    partial = {name: None for name in C_SUMS}
    missing = {name: len(terms) for name, terms in C_SUMS.items()}
    for r in order:
        arrived = [("p%d" % r, product(r))]
        while arrived:
            term, v = arrived.pop(0)
            for name, terms in C_SUMS.items():
                if term not in terms:
                    continue
                sign = terms[term]
                if partial[name] is None:
                    partial[name] = (sign, v)
                else:
                    s0, v0 = partial[name]
                    partial[name] = (s0, v0 + v) if s0 == sign else (1, v0 - v if s0 > 0 else v - v0)
                missing[name] -= 1
                if missing[name] == 0:
                    assert partial[name][0] > 0
                    if name[0] == "t":
                        arrived.append((name, partial[name][1]))
                    else:
                        yield int(name[1]), partial[name][1]


def signed_sum(coefs, get):
    acc = None
    for j, c in enumerate(coefs):
        if c:
            v = get(j)
            acc = (v if c > 0 else -v) if acc is None else (acc + v if c > 0 else acc - v)
    return acc


ORDER1 = (10, 12, 14, 9, 1, 2, 6, 11, 13, 0, 3, 7, 8, 4, 5)
ORDER2 = (1, 2, 3, 0, 10, 12, 14, 9, 6, 11, 13, 7, 8, 4, 5)


def make(TM=1536, TC=384, US=16, NL=3, M2=32, NH=3, NX=4, ND=3,  ord1=ORDER1, ord2=ORDER2,
         only=None, flags=None, nobc=True):
    TH = TM - TC

    def kernel(x_hbm, dw_hbm, w1_hbm, w2_hbm, g_ref, b_ref, o_hbm, h_hbm,
               xbuf, hbuf, hcache, wc, fbuf, ybuf, ssq, dw_ref, w2_ref, sem_x, sem_h, sem_w):
        N, C = x_hbm.shape
        D = w1_hbm.shape[1]
        NB = N // TM
        NT = D // 128
        G = NT // 3

        def x_in(i):
            return pltpu.make_async_copy(x_hbm.at[pl.ds(i * TM, TM)], xbuf.at[x_slot(i)], sem_x.at[x_slot(i)])

        def o_out(i):
            return pltpu.make_async_copy(xbuf.at[x_slot(i)], o_hbm.at[pl.ds(i * TM, TM)], sem_x.at[x_slot(i)])

        def h_out(i, hs):
            return pltpu.make_async_copy(hbuf.at[hs], h_hbm.at[i - NH], sem_h.at[hs])

        def h_in(i, hs):
            return pltpu.make_async_copy(h_hbm.at[i - NH], hbuf.at[hs], sem_h.at[hs])

        def h_place(i, hs, r0):
            return (hcache, i, r0 - TH) if r0 >= TH else (hbuf, hs, r0)

        def x_slot(i):
            return jnp.bitwise_and(i, NX - 1)

        def weight(r, q):
            return pltpu.bitcast(wc[r, q], BF16)

        def layernorm(slot, starts):
            dw = dw_ref[...].astype(F32)
            xc, ss = [], []
            for r0 in starts:
                xv = xbuf[slot, pl.ds(r0, 8), :].astype(F32) * dw
                xc.append(xv - jnp.sum(xv, axis=-1, keepdims=True) * (1.0 / C))
                ss.append(jnp.sum(xc[-1] * xc[-1], axis=-1, keepdims=True))
            inv_std = lambda v: jax.lax.rsqrt(v * (1.0 / (C * ALPHA * ALPHA)) + 1e-5 / (ALPHA * ALPHA))
            return [v * inv_std(t) for v, t in zip(xc, ss)]

        def left_unit(slot, u):
            groups = range(0, US, 8)
            a = layernorm(slot, [(2 * u + half) * US + k for k in groups for half in range(2)])
            forms = [a_forms([v[:, k * 128:(k + 1) * 128] for v in a[2 * g:2 * g + 2] for k in range(3)])
                     for g in range(len(groups))]
            return [jnp.concatenate([f[r] for f in forms], axis=0) for r in range(15)]

        def activate(y, places, c, q, acc):
            n = (c % 3) * G + q
            h = y + y * jnp.tanh(y * (y * y + BETA))
            sq = h * h
            for k in range(0, y.shape[0], 8):
                acc[n] = sq[k:k + 8] if acc[n] is None else acc[n] + sq[k:k + 8]
            hb = h.astype(BF16)
            for k, (i, hs, u) in enumerate(places):
                ref, j, r = h_place(i, hs, (2 * u + c // 3) * US)
                ref[j, n, pl.ds(r, US), :] = hb[k * US:(k + 1) * US]

        def flush(acc):
            for n, v in enumerate(acc):
                if v is not None:
                    ssq[:, n * 128:(n + 1) * 128] += v

        def first_matmul(units, q):
            def product(r):
                fresh = [u[r] for u in units if u[r].dtype == F32]
                lhs = [u[r] for u in units if u[r].dtype == BF16]
                if fresh:
                    lhs.append(jnp.concatenate(fresh, axis=0).astype(BF16))
                return jnp.dot(jnp.concatenate(lhs, axis=0), weight(r, q), preferred_element_type=F32)
            return block_products(ord1, product)

        NU = TM // (2 * US)
        NS = NU * G // NL
        live_at = lambda t: [u for u in range(1 - NL, NU) if 0 <= t - (G * u) // NL < G]
        done_order = [c for c, _ in block_products(ord1, lambda r: 0.0)]
        deferred = done_order[6 - ND:] if ND else []

        def activate_deferred(i, acc):
            for k, c in enumerate(deferred):
                activate(ybuf[k], [(i, None, u) for u in live_at(NS - 1)], c, (NS - 1) % G, acc)

        def pass1(step, hs):
            i = NB - 1 - step

            @pl.when(i >= NX - 1)
            def _():
                x_in(i - (NX - 1)).start()

            @pl.when(i >= 1)
            def _():
                x_in(i - 1).wait()

            @pl.when(i + NH < NB)
            def _():
                h_out(i + NH, hs).wait()

            acc = [None] * NT
            prev = jnp.minimum(i + 1, NB - 1)
            activate_deferred(prev, acc)
            units = {k - (NL - 1): [fbuf[k, r] for r in range(15)] for k in range(NL)}
            for t in range(NS):
                for u in (live_at(t + 1) if t + 1 < NS else [NU]):
                    if u not in units:
                        units[u] = left_unit(x_slot(i), u) if u < NU else left_unit(x_slot(jnp.maximum(i - 1, 0)), 0)
                live = live_at(t)
                for c, y in first_matmul([units[u] for u in live], t % G):
                    if t == NS - 1 and c in deferred:
                        ybuf[deferred.index(c)] = y
                    else:
                        activate(y, [(i, hs, u) if u >= 0 else (prev, None, u + NU) for u in live], c, t % G, acc)
            for k in range(NL):
                for r in range(15):
                    fbuf[k, r] = units[NU - (NL - 1) + k][r].astype(BF16)
            flush(acc)

            @pl.when(i >= NH)
            def _():
                h_out(i, hs).start()

            return jnp.where(hs == 0, NH - 1, hs - 1)

        w2_in = pltpu.make_async_copy(w2_hbm, w2_ref, sem_w.at[1])
        if only != 2:
            w1_in = [pltpu.make_async_copy(w1_hbm.at[pl.ds(k * 128, 128), pl.ds(n * 128, 128)],
                                           hcache.at[k, n, pl.ds(0, 128)], sem_w.at[0])
                     for k in range(3) for n in range(NT)]
            w1_in.append(pltpu.make_async_copy(dw_hbm, dw_ref, sem_w.at[0]))
            for cp in w1_in:
                cp.start()
            x_in(NB - 1).start()
            ssq[...] = jnp.zeros_like(ssq)
            ybuf[...] = jnp.zeros_like(ybuf)
            fbuf[...] = jnp.zeros_like(fbuf)
            for cp in w1_in:
                cp.wait()
            for q in range(G):
                w1_block = lambda j: hcache[j // 3, (j % 3) * G + q, pl.ds(0, 128), :].astype(F32)
                for r in range(15):
                    wc[r, q] = pltpu.bitcast(signed_sum(B_FORMS[r], w1_block).astype(BF16), U32)
            x_in(NB - 1).wait()
            for s in range(1, NX - 1):
                x_in(NB - 1 - s).start()
            w2_in.start()
            for r, f in enumerate(left_unit((NB - 1) % NX, 0)):
                fbuf[NL - 1, r] = f.astype(BF16)
            jax.lax.fori_loop(0, NB, pass1, jnp.int32((NB - 1) % NH))
            acc = [None] * NT
            activate_deferred(0, acc)
            for t in range(G - 1):
                live = [u for u in live_at(t) if u < 0]
                if live:
                    for c, y in first_matmul([[fbuf[u + NL - 1, r] for r in range(15)] for u in live], t):
                        activate(y, [(0, None, NU + u) for u in live], c, t, acc)
            flush(acc)
        if only == 2:
            w2_in.start()
        w2_in.wait()
        if only == 1:
            return
        if only == 2:
            for s in range(NX):
                x_in(s).start()
                x_in(s).wait()

        gx = jnp.sqrt(jnp.sum(ssq[...], axis=0, keepdims=True) * (HSCALE * HSCALE) + 1e-6)
        nx = gx / (jnp.mean(gx, axis=-1, keepdims=True) + 1e-6)
        scale = (1.0 + g_ref[...].astype(F32).reshape(1, D) * nx) * HSCALE
        b_row = b_ref[...].astype(F32).reshape(1, D)
        bias = jnp.dot(jnp.broadcast_to(b_row, (16, D)).astype(BF16), w2_ref[...], preferred_element_type=F32)[0:1]
        for q in range(G):
            col = [jnp.broadcast_to(scale[:, (k * G + q) * 128:(k * G + q + 1) * 128], (128, 128)).T for k in range(3)]
            blocks = [w2_ref[pl.ds(((j // 3) * G + q) * 128, 128), pl.ds((j % 3) * 128, 128)].astype(F32) * col[j // 3]
                      for j in range(9)]
            for r in range(15):
                wc[r, q] = pltpu.bitcast(signed_sum(B_FORMS[r], blocks.__getitem__).astype(BF16), U32)

        def pass2(i, hs):
            @pl.when(i >= 2)
            def _():
                o_out(i - 2).wait()

            @pl.when(jnp.logical_and(i >= 2, i + NX - 2 < NB))
            def _():
                x_in(i + NX - 2).start()


            @pl.when(i >= NH)
            def _():
                h_in(i, hs).wait()

            @pl.when(i >= NX)
            def _():
                x_in(i).wait()

            for r0 in range(0, TM, 2 * M2):
                if r0 == TH:
                    @pl.when(i + NH < NB)
                    def _():
                        h_in(i + NH, hs).start()

                raw = []
                for half in range(2):
                    ref, j, r = h_place(i, hs, r0 + half * M2)
                    raw += [jnp.concatenate([ref[j, k * G + q, pl.ds(r, M2), :] for q in range(G)], axis=1)
                            for k in range(3)]
                forms = a_forms([v.astype(F32) for v in raw])
                forms = [raw[4], raw[1], raw[2], raw[3]] + [f.astype(BF16) for f in forms[4:]]
                product = lambda r: jnp.dot(
                    forms[r], jnp.concatenate([weight(r, q) for q in range(G)], axis=0), preferred_element_type=F32)
                for c, y in block_products(ord2, product):
                    rows = pl.ds(r0 + (c // 3) * M2, M2)
                    cols = slice((c % 3) * 128, (c % 3 + 1) * 128)
                    xbuf[x_slot(i), rows, cols] = (y + bias[:, cols] + xbuf[x_slot(i), rows, cols].astype(F32)).astype(BF16)
            o_out(i).start()
            return jnp.where(hs == NH - 1, 0, hs + 1)

        jax.lax.fori_loop(0, NB, pass2, jnp.int32(0))
        o_out(NB - 2).wait()
        o_out(NB - 1).wait()

    def fn(x, dw, w1, w2, grn_g, grn_b):
        B, H, W, C = x.shape
        N = B * H * W
        D = w1.shape[1]
        NB = N // TM
        NT = D // 128
        assert (TM // (2 * US) * (NT // 3)) % NL == 0
        assert B == 1 and dw.shape[:2] == (1, 1) and C == 384 and D % 384 == 0 and N % TM == 0
        hbm = pl.BlockSpec(memory_space=pl.ANY)
        vmem = pl.BlockSpec(memory_space=pltpu.VMEM)
        out, _ = pl.pallas_call(
            kernel,
            in_specs=[hbm, hbm, hbm, hbm, vmem, vmem],
            out_specs=[hbm, hbm],
            out_shape=[jax.ShapeDtypeStruct((N, C), x.dtype), jax.ShapeDtypeStruct((NB - NH, NT, TH, 128), BF16)],
            scratch_shapes=[
                pltpu.VMEM((NX, TM, C), BF16),
                pltpu.VMEM((NH, NT, TH, 128), BF16),
                pltpu.VMEM((NB, NT, TC, 128), BF16),
                pltpu.VMEM((15, NT // 3, 64, 128), U32),
                pltpu.VMEM((NL, 15, US, 128), BF16),
                pltpu.VMEM((max(ND, 1), NL * US, 128), F32),
                pltpu.VMEM((8, D), F32),
                pltpu.VMEM((1, C), dw.dtype),
                pltpu.VMEM((D, C), w2.dtype),
                pltpu.SemaphoreType.DMA((NX,)),
                pltpu.SemaphoreType.DMA((NH,)),
                pltpu.SemaphoreType.DMA((2,)),
            ],
            compiler_params=pltpu.CompilerParams(
                vmem_limit_bytes=128 * 1024 * 1024, flags=flags, disable_bounds_checks=nobc),
        )(x.reshape(N, C), dw.reshape(1, C), w1, w2, grn_g, grn_b)
        return out.reshape(x.shape)

    return fn


@jax.jit
def pallas_standalone__modern_conv_block_slak__vision_kernel(x, dw, w1, w2, grn_g, grn_b):
    return make()(x, dw, w1, w2, grn_g, grn_b)
```

```python
import numpy as np
import jax
import jax.numpy as jnp
import jax.experimental.pallas as pl
import jax.experimental.pallas.tpu as pltpu

F32 = jnp.float32
BF16 = jnp.bfloat16
U32 = jnp.uint32

_C0 = float(np.sqrt(2.0 / np.pi))
ALPHA = float((_C0 * 0.044715) ** (1.0 / 3.0))
BETA = _C0 / ALPHA
HSCALE = 0.5 / ALPHA

B_FORMS = (
    (0, 0, 0, -1, 1, 0, -1, 0, 0),
    (-1, 0, 0, -1, 0, 1, 0, 0, 0),
    (0, 0, -1, 0, 0, 0, -1, 0, 1),
    (1, -1, 0, 0, 0, 0, 0, 1, 0),
    (0, 0, 0, 0, 0, -1, 0, -1, -1),
    (0, -1, -1, 0, -1, 0, 0, 0, 0),
    (0, 0, 1, 0, 0, 0, 0, 0, 0),
    (0, 0, 0, 0, 0, 0, 0, -1, 0),
    (0, 0, -1, 0, 0, 0, 0, -1, 0),
    (-1, 0, 0, 0, 0, 0, 0, 0, 0),
    (0, 0, 0, 0, 0, 0, -1, 0, 0),
    (1, 0, 0, 0, 1, 0, 0, 0, 0),
    (0, 0, 0, 0, 0, 1, 1, 0, 0),
    (0, 0, 0, 0, -1, 0, 0, 0, 0),
    (0, 0, 0, 0, 0, -1, 0, 0, 0),
)


def a_forms(a):
    a0, a1, a2, a3, a4, a5 = a
    d54 = a5 - a4
    d10 = a1 - a0
    e = a3 - d10
    f = d54 + a2
    return [a4, a1, a2, a3, a2 + a5, a0 + a3, a0 + a2, a3 + a5, a3 - a2, d10, d54, e, f, a4 - e, a1 - f]


C_SUMS = {
    "t1": {"p10": 1, "p12": 1},
    "t2": {"t1": 1, "p14": -1},
    "t3": {"p11": 1, "p9": -1},
    "t4": {"t3": 1, "p13": -1},
    "c0": {"t2": 1, "p9": 1, "p1": -1},
    "c1": {"p3": 1, "t3": -1, "p6": -1, "p8": 1, "p5": -1},
    "c2": {"t2": 1, "p2": 1, "p6": 1},
    "c3": {"t4": 1, "p10": -1, "p0": -1},
    "c4": {"t4": 1, "p3": -1, "p7": -1},
    "c5": {"p7": 1, "t1": -1, "p2": -1, "p8": -1, "p4": -1},
}


def block_products(order, product):
    partial = {name: None for name in C_SUMS}
    missing = {name: len(terms) for name, terms in C_SUMS.items()}
    for r in order:
        arrived = [("p%d" % r, product(r))]
        while arrived:
            term, v = arrived.pop(0)
            for name, terms in C_SUMS.items():
                if term not in terms:
                    continue
                sign = terms[term]
                if partial[name] is None:
                    partial[name] = (sign, v)
                else:
                    s0, v0 = partial[name]
                    partial[name] = (s0, v0 + v) if s0 == sign else (1, v0 - v if s0 > 0 else v - v0)
                missing[name] -= 1
                if missing[name] == 0:
                    assert partial[name][0] > 0
                    if name[0] == "t":
                        arrived.append((name, partial[name][1]))
                    else:
                        yield int(name[1]), partial[name][1]


def signed_sum(coefs, get):
    acc = None
    for j, c in enumerate(coefs):
        if c:
            v = get(j)
            acc = (v if c > 0 else -v) if acc is None else (acc + v if c > 0 else acc - v)
    return acc


ORDER1 = (10, 12, 14, 9, 1, 2, 6, 11, 13, 0, 3, 7, 8, 4, 5)
ORDER2 = (1, 2, 3, 0, 10, 12, 14, 9, 6, 11, 13, 7, 8, 4, 5)


def make(TM=1536, TC=384, US=16, NL=3, M2=32, NH=3, NP=1, MID=True, RR=128, RP=64, NX=4, ND=3,  ord1=ORDER1, ord2=ORDER2,
         only=None, flags=None, nobc=True):
    TH = TM - TC
    TP = TH // NP
    assert TH % NP == 0 and TP % (2 * M2) == 0 and TP % US == 0 and (MID or NP == 1)
    assert RP % (2 * M2) == 0 and RP < TH - RR and RR % (2 * US) == 0

    def kernel(x_hbm, dw_hbm, w1_hbm, w2_hbm, g_ref, b_ref, o_hbm, h_hbm,
               xbuf, hbuf, hcache, wc, w1_last, fbuf, ybuf, ssq, dw_ref, w2_ref, sem_x, sem_h, sem_w):
        N, C = x_hbm.shape
        D = w1_hbm.shape[1]
        NB = N // TM
        NT = D // 128
        G = NT // 3

        def x_in(i):
            return pltpu.make_async_copy(x_hbm.at[pl.ds(i * TM, TM)], xbuf.at[x_slot(i)], sem_x.at[x_slot(i)])

        def o_out(i):
            return pltpu.make_async_copy(xbuf.at[x_slot(i)], o_hbm.at[pl.ds(i * TM, TM)], sem_x.at[x_slot(i)])

        def h_out(i, hs):
            return pltpu.make_async_copy(hbuf.at[hs], h_hbm.at[i - NH], sem_h.at[hs, 0])

        def h_in(i, hs, k):
            if k < NP - 1 or not RR:
                pieces = [(k,)]
            else:
                pieces = [(k, pl.ds(0, NT - 3))] + ([(k, pl.ds(NT - 3, 3), pl.ds(0, TP - RR))] if RR < TP else [])
            return [pltpu.make_async_copy(h_hbm.at[(i - NH, *p)], hbuf.at[(hs, *p)], sem_h.at[hs, k]) for p in pieces]

        def h_place(i, hs, r0):
            return (hcache, (i,), r0 - TH) if r0 >= TH else (hbuf, (hs, r0 // TP), r0 % TP)

        def x_slot(i):
            return jnp.bitwise_and(i, NX - 1)

        def weight(r, q):
            return pltpu.bitcast(wc[r, q], BF16)

        def layernorm(slot, starts):
            dw = dw_ref[...].astype(F32)
            xc, ss = [], []
            for r0 in starts:
                xv = xbuf[slot, pl.ds(r0, 8), :].astype(F32) * dw
                xc.append(xv - jnp.sum(xv, axis=-1, keepdims=True) * (1.0 / C))
                ss.append(jnp.sum(xc[-1] * xc[-1], axis=-1, keepdims=True))
            inv_std = lambda v: jax.lax.rsqrt(v * (1.0 / (C * ALPHA * ALPHA)) + 1e-5 / (ALPHA * ALPHA))
            return [v * inv_std(t) for v, t in zip(xc, ss)]

        def left_unit(slot, u):
            groups = range(0, US, 8)
            a = layernorm(slot, [(2 * u + half) * US + k for k in groups for half in range(2)])
            forms = [a_forms([v[:, k * 128:(k + 1) * 128] for v in a[2 * g:2 * g + 2] for k in range(3)])
                     for g in range(len(groups))]
            return [jnp.concatenate([f[r] for f in forms], axis=0) for r in range(15)]

        def activate(y, places, c, q, acc):
            n = 3 * q + c % 3
            h = y + y * jnp.tanh(y * (y * y + BETA))
            if acc is not None:
                sq = h * h
                for k in range(0, y.shape[0], 8):
                    acc[n] = sq[k:k + 8] if acc[n] is None else acc[n] + sq[k:k + 8]
            hb = h.astype(BF16)
            for k, (i, hs, u) in enumerate(places):
                ref, j, r = h_place(i, hs, (2 * u + c // 3) * US)
                ref[(*j, n, pl.ds(r, US), slice(None))] = hb[k * US:(k + 1) * US]

        def flush(acc):
            for n, v in enumerate(acc):
                if v is not None:
                    col = ((n % 3) * G + n // 3) * 128
                    ssq[:, col:col + 128] += v

        def first_matmul(units, rhs):
            def product(r):
                fresh = [u[r] for u in units if u[r].dtype == F32]
                lhs = [u[r] for u in units if u[r].dtype == BF16]
                if fresh:
                    lhs.append(jnp.concatenate(fresh, axis=0).astype(BF16))
                return jnp.dot(jnp.concatenate(lhs, axis=0), rhs(r), preferred_element_type=F32)
            return block_products(ord1, product)

        NU = TM // (2 * US)
        NS = NU * G // NL
        live_at = lambda t: [u for u in range(1 - NL, NU) if 0 <= t - (G * u) // NL < G]
        done_order = [c for c, _ in block_products(ord1, lambda r: 0.0)]
        deferred = done_order[6 - ND:] if ND else []

        def activate_deferred(i, acc):
            for k, c in enumerate(deferred):
                activate(ybuf[k], [(i, None, u) for u in live_at(NS - 1)], c, (NS - 1) % G, acc)

        def pass1(step, hs):
            i = NB - 1 - step

            @pl.when(i >= NX - 1)
            def _():
                x_in(i - (NX - 1)).start()

            @pl.when(i >= 1)
            def _():
                x_in(i - 1).wait()

            @pl.when(i + NH < NB)
            def _():
                h_out(i + NH, hs).wait()

            acc = [None] * NT
            prev = jnp.minimum(i + 1, NB - 1)
            activate_deferred(prev, acc)
            units = {k - (NL - 1): [fbuf[k, r] for r in range(15)] for k in range(NL)}
            for t in range(NS):
                for u in (live_at(t + 1) if t + 1 < NS else [NU]):
                    if u not in units:
                        units[u] = left_unit(x_slot(i), u) if u < NU else left_unit(x_slot(jnp.maximum(i - 1, 0)), 0)
                live = live_at(t)
                for c, y in first_matmul([units[u] for u in live], lambda r: weight(r, t % G)):
                    if t == NS - 1 and c in deferred:
                        ybuf[deferred.index(c)] = y
                    else:
                        activate(y, [(i, hs, u) if u >= 0 else (prev, None, u + NU) for u in live], c, t % G, acc)
            for k in range(NL):
                for r in range(15):
                    fbuf[k, r] = units[NU - (NL - 1) + k][r].astype(BF16)
            flush(acc)

            @pl.when(i >= NH)
            def _():
                h_out(i, hs).start()

            return jnp.where(hs == 0, NH - 1, hs - 1)

        w2_in = pltpu.make_async_copy(w2_hbm, w2_ref, sem_w.at[1])
        if only != 2:
            w1_in = [pltpu.make_async_copy(w1_hbm.at[pl.ds(k * 128, 128), pl.ds(n * 128, 128)],
                                           hcache.at[k, n, pl.ds(0, 128)], sem_w.at[0])
                     for k in range(3) for n in range(NT)]
            w1_in.append(pltpu.make_async_copy(dw_hbm, dw_ref, sem_w.at[0]))
            for cp in w1_in:
                cp.start()
            x_in(NB - 1).start()
            ssq[...] = jnp.zeros_like(ssq)
            ybuf[...] = jnp.zeros_like(ybuf)
            fbuf[...] = jnp.zeros_like(fbuf)
            for cp in w1_in:
                cp.wait()
            for q in range(G):
                w1_block = lambda j: hcache[j // 3, (j % 3) * G + q, pl.ds(0, 128), :].astype(F32)
                for r in range(15):
                    wc[r, q] = pltpu.bitcast(signed_sum(B_FORMS[r], w1_block).astype(BF16), U32)
            x_in(NB - 1).wait()
            for s in range(1, NX - 1):
                x_in(NB - 1 - s).start()
            w2_in.start()
            for r, f in enumerate(left_unit((NB - 1) % NX, 0)):
                fbuf[NL - 1, r] = f.astype(BF16)
            jax.lax.fori_loop(0, NB, pass1, jnp.int32((NB - 1) % NH))
            acc = [None] * NT
            activate_deferred(0, acc)
            for t in range(G - 1):
                live = [u for u in live_at(t) if u < 0]
                if live:
                    for c, y in first_matmul([[fbuf[u + NL - 1, r] for r in range(15)] for u in live], lambda r: weight(r, t)):
                        activate(y, [(0, None, NU + u) for u in live], c, t, acc)
            flush(acc)
        if only == 2:
            w2_in.start()
        w2_in.wait()
        if only == 1:
            return
        if only == 2:
            for s in range(NX):
                x_in(s).start()
                x_in(s).wait()

        gx = jnp.sqrt(jnp.sum(ssq[...], axis=0, keepdims=True) * (HSCALE * HSCALE) + 1e-6)
        nx = gx / (jnp.mean(gx, axis=-1, keepdims=True) + 1e-6)
        scale = (1.0 + g_ref[...].astype(F32).reshape(1, D) * nx) * HSCALE
        b_row = b_ref[...].astype(F32).reshape(1, D)
        bias = jnp.dot(jnp.broadcast_to(b_row, (16, D)).astype(BF16), w2_ref[...], preferred_element_type=F32)[0:1]
        w1_last[...] = wc[:, G - 1]
        for q in range(G):
            col = [jnp.broadcast_to(scale[:, (k * G + q) * 128:(k * G + q + 1) * 128], (128, 128)).T for k in range(3)]
            blocks = [w2_ref[pl.ds(((j // 3) * G + q) * 128, 128), pl.ds((j % 3) * 128, 128)].astype(F32) * col[j // 3]
                      for j in range(9)]
            for r in range(15):
                wc[r, q] = pltpu.bitcast(signed_sum(B_FORMS[r], blocks.__getitem__).astype(BF16), U32)

        def pass2(i, hs):
            @pl.when(i >= 2)
            def _():
                o_out(i - 2).wait()

            @pl.when(jnp.logical_and(i >= 2, i + NX - 2 < NB))
            def _():
                x_in(i + NX - 2).start()


            if not MID:
                @pl.when(jnp.logical_and(i >= 1, i + NH - 1 < NB))
                def _():
                    for cp in h_in(i + NH - 1, jnp.where(hs == 0, NH - 1, hs - 1), 0):
                        cp.start()

            @pl.when(i >= NH)
            def _():
                for cp in h_in(i, hs, 0):
                    cp.wait()

            @pl.when(i >= NX)
            def _():
                x_in(i).wait()

            for r0 in range(0, TM, 2 * M2):
                if RR and r0 == RP:
                    redo = range((TH - RR) // (2 * US), TH // (2 * US))
                    for c, y in first_matmul([left_unit(x_slot(i), u) for u in redo],
                                             lambda r: pltpu.bitcast(w1_last[r], BF16)):
                        activate(y, [(i, hs, u) for u in redo], c, G - 1, None)
                if MID and 0 < r0 <= TH and r0 % TP == 0:
                    @pl.when(i + NH < NB)
                    def _():
                        for cp in h_in(i + NH, hs, r0 // TP - 1):
                            cp.start()

                    if r0 < TH:
                        @pl.when(i >= NH)
                        def _():
                            for cp in h_in(i, hs, r0 // TP):
                                cp.wait()

                raw = []
                for half in range(2):
                    ref, j, r = h_place(i, hs, r0 + half * M2)
                    raw += [jnp.concatenate([ref[(*j, 3 * q + k, pl.ds(r, M2), slice(None))] for q in range(G)], axis=1)
                            for k in range(3)]
                forms = a_forms([v.astype(F32) for v in raw])
                forms = [raw[4], raw[1], raw[2], raw[3]] + [f.astype(BF16) for f in forms[4:]]
                product = lambda r: jnp.dot(
                    forms[r], jnp.concatenate([weight(r, q) for q in range(G)], axis=0), preferred_element_type=F32)
                for c, y in block_products(ord2, product):
                    rows = pl.ds(r0 + (c // 3) * M2, M2)
                    cols = slice((c % 3) * 128, (c % 3 + 1) * 128)
                    xbuf[x_slot(i), rows, cols] = (y + bias[:, cols] + xbuf[x_slot(i), rows, cols].astype(F32)).astype(BF16)
            o_out(i).start()
            return jnp.where(hs == NH - 1, 0, hs + 1)

        jax.lax.fori_loop(0, NB, pass2, jnp.int32(0))
        o_out(NB - 2).wait()
        o_out(NB - 1).wait()

    def fn(x, dw, w1, w2, grn_g, grn_b):
        B, H, W, C = x.shape
        N = B * H * W
        D = w1.shape[1]
        NB = N // TM
        NT = D // 128
        assert (TM // (2 * US) * (NT // 3)) % NL == 0
        assert B == 1 and dw.shape[:2] == (1, 1) and C == 384 and D % 384 == 0 and N % TM == 0
        hbm = pl.BlockSpec(memory_space=pl.ANY)
        vmem = pl.BlockSpec(memory_space=pltpu.VMEM)
        out, _ = pl.pallas_call(
            kernel,
            in_specs=[hbm, hbm, hbm, hbm, vmem, vmem],
            out_specs=[hbm, hbm],
            out_shape=[jax.ShapeDtypeStruct((N, C), x.dtype), jax.ShapeDtypeStruct((NB - NH, NP, NT, TP, 128), BF16)],
            scratch_shapes=[
                pltpu.VMEM((NX, TM, C), BF16),
                pltpu.VMEM((NH, NP, NT, TP, 128), BF16),
                pltpu.VMEM((NB, NT, TC, 128), BF16),
                pltpu.VMEM((15, NT // 3, 64, 128), U32),
                pltpu.VMEM((15, 64, 128), U32),
                pltpu.VMEM((NL, 15, US, 128), BF16),
                pltpu.VMEM((max(ND, 1), NL * US, 128), F32),
                pltpu.VMEM((8, D), F32),
                pltpu.VMEM((1, C), dw.dtype),
                pltpu.VMEM((D, C), w2.dtype),
                pltpu.SemaphoreType.DMA((NX,)),
                pltpu.SemaphoreType.DMA((NH, NP)),
                pltpu.SemaphoreType.DMA((2,)),
            ],
            compiler_params=pltpu.CompilerParams(
                vmem_limit_bytes=128 * 1024 * 1024, flags=flags, disable_bounds_checks=nobc),
        )(x.reshape(N, C), dw.reshape(1, C), w1, w2, grn_g, grn_b)
        return out.reshape(x.shape)

    return fn


@jax.jit
def pallas_standalone__modern_conv_block_slak__vision_kernel(x, dw, w1, w2, grn_g, grn_b):
    return make()(x, dw, w1, w2, grn_g, grn_b)
```

```python
import numpy as np
import jax
import jax.numpy as jnp
import jax.experimental.pallas as pl
import jax.experimental.pallas.tpu as pltpu

F32 = jnp.float32
BF16 = jnp.bfloat16
U32 = jnp.uint32

_C0 = float(np.sqrt(2.0 / np.pi))
ALPHA = float((_C0 * 0.044715) ** (1.0 / 3.0))
BETA = _C0 / ALPHA
HSCALE = 0.5 / ALPHA

TM = 1536
TC = 384
TH = TM - TC
NH = 3
NX = 4
US = 16
NL = 3
ND = 3
M2 = 32
RR = 128
RP = 64

B_FORMS = (
    (0, 0, 0, -1, 1, 0, -1, 0, 0),
    (-1, 0, 0, -1, 0, 1, 0, 0, 0),
    (0, 0, -1, 0, 0, 0, -1, 0, 1),
    (1, -1, 0, 0, 0, 0, 0, 1, 0),
    (0, 0, 0, 0, 0, -1, 0, -1, -1),
    (0, -1, -1, 0, -1, 0, 0, 0, 0),
    (0, 0, 1, 0, 0, 0, 0, 0, 0),
    (0, 0, 0, 0, 0, 0, 0, -1, 0),
    (0, 0, -1, 0, 0, 0, 0, -1, 0),
    (-1, 0, 0, 0, 0, 0, 0, 0, 0),
    (0, 0, 0, 0, 0, 0, -1, 0, 0),
    (1, 0, 0, 0, 1, 0, 0, 0, 0),
    (0, 0, 0, 0, 0, 1, 1, 0, 0),
    (0, 0, 0, 0, -1, 0, 0, 0, 0),
    (0, 0, 0, 0, 0, -1, 0, 0, 0),
)


def a_forms(a):
    a0, a1, a2, a3, a4, a5 = a
    d54 = a5 - a4
    d10 = a1 - a0
    e = a3 - d10
    f = d54 + a2
    return [a4, a1, a2, a3, a2 + a5, a0 + a3, a0 + a2, a3 + a5, a3 - a2, d10, d54, e, f, a4 - e, a1 - f]


C_SUMS = {
    "t1": {"p10": 1, "p12": 1},
    "t2": {"t1": 1, "p14": -1},
    "t3": {"p11": 1, "p9": -1},
    "t4": {"t3": 1, "p13": -1},
    "c0": {"t2": 1, "p9": 1, "p1": -1},
    "c1": {"p3": 1, "t3": -1, "p6": -1, "p8": 1, "p5": -1},
    "c2": {"t2": 1, "p2": 1, "p6": 1},
    "c3": {"t4": 1, "p10": -1, "p0": -1},
    "c4": {"t4": 1, "p3": -1, "p7": -1},
    "c5": {"p7": 1, "t1": -1, "p2": -1, "p8": -1, "p4": -1},
}

ORDER1 = (10, 12, 14, 9, 1, 2, 6, 11, 13, 0, 3, 7, 8, 4, 5)
ORDER2 = (1, 2, 3, 0, 10, 12, 14, 9, 6, 11, 13, 7, 8, 4, 5)


def block_products(order, product):
    partial = {name: None for name in C_SUMS}
    missing = {name: len(terms) for name, terms in C_SUMS.items()}
    for r in order:
        arrived = [("p%d" % r, product(r))]
        while arrived:
            term, v = arrived.pop(0)
            for name, terms in C_SUMS.items():
                if term not in terms:
                    continue
                sign = terms[term]
                if partial[name] is None:
                    partial[name] = (sign, v)
                else:
                    s0, v0 = partial[name]
                    partial[name] = (s0, v0 + v) if s0 == sign else (1, v0 - v if s0 > 0 else v - v0)
                missing[name] -= 1
                if missing[name] == 0:
                    assert partial[name][0] > 0
                    if name[0] == "t":
                        arrived.append((name, partial[name][1]))
                    else:
                        yield int(name[1]), partial[name][1]


def signed_sum(coefs, get):
    acc = None
    for j, c in enumerate(coefs):
        if c:
            v = get(j)
            acc = (v if c > 0 else -v) if acc is None else (acc + v if c > 0 else acc - v)
    return acc


def _kernel(x_hbm, dw_hbm, w1_hbm, w2_hbm, g_ref, b_ref, o_hbm, h_hbm,
            xbuf, hbuf, hcache, wc, fbuf, ybuf, ssq, dw_ref, aux, sem_x, sem_h, sem_w):
    N, C = x_hbm.shape
    D = w1_hbm.shape[1]
    NB = N // TM
    NT = D // 128
    G = NT // 3

    def x_slot(i):
        return i & (NX - 1)

    def x_in(i):
        return pltpu.make_async_copy(x_hbm.at[pl.ds(i * TM, TM)], xbuf.at[x_slot(i)], sem_x.at[x_slot(i)])

    def o_out(i):
        return pltpu.make_async_copy(xbuf.at[x_slot(i)], o_hbm.at[pl.ds(i * TM, TM)], sem_x.at[x_slot(i)])

    def h_out(i, hs):
        return pltpu.make_async_copy(hbuf.at[hs], h_hbm.at[i - NH], sem_h.at[hs])

    def h_in(i, hs):
        pieces = ((pl.ds(0, NT - 3),), (pl.ds(NT - 3, 3), pl.ds(0, TH - RR)))
        return [pltpu.make_async_copy(h_hbm.at[(i - NH, *p)], hbuf.at[(hs, *p)], sem_h.at[hs]) for p in pieces]

    def h_place(i, hs, r0):
        return (hcache, i, r0 - TH) if r0 >= TH else (hbuf, hs, r0)

    def weight(r, q):
        return pltpu.bitcast(wc[r, q], BF16)

    def left_unit(slot, u):
        dw = dw_ref[...].astype(F32)
        groups = range(0, US, 8)
        xc, ss = [], []
        for r0 in [(2 * u + half) * US + k for k in groups for half in range(2)]:
            xv = xbuf[slot, pl.ds(r0, 8), :].astype(F32) * dw
            xc.append(xv - jnp.sum(xv, axis=-1, keepdims=True) * (1.0 / C))
            ss.append(jnp.sum(xc[-1] * xc[-1], axis=-1, keepdims=True))
        a = [v * jax.lax.rsqrt(t * (1.0 / (C * ALPHA * ALPHA)) + 1e-5 / (ALPHA * ALPHA)) for v, t in zip(xc, ss)]
        forms = [a_forms([v[:, k * 128:(k + 1) * 128] for v in a[2 * g:2 * g + 2] for k in range(3)])
                 for g in range(len(groups))]
        return [jnp.concatenate([f[r] for f in forms], axis=0) for r in range(15)]

    def first_matmul(units, rhs):
        def product(r):
            fresh = [u[r] for u in units if u[r].dtype == F32]
            lhs = [u[r] for u in units if u[r].dtype == BF16]
            if fresh:
                lhs.append(jnp.concatenate(fresh, axis=0).astype(BF16))
            return jnp.dot(jnp.concatenate(lhs, axis=0), rhs(r), preferred_element_type=F32)
        return block_products(ORDER1, product)

    def activate(y, places, c, q, acc):
        n = 3 * q + c % 3
        h = y + y * jnp.tanh(y * (y * y + BETA))
        if acc is not None:
            sq = h * h
            for k in range(0, y.shape[0], 8):
                acc[n] = sq[k:k + 8] if acc[n] is None else acc[n] + sq[k:k + 8]
        hb = h.astype(BF16)
        for k, (i, hs, u) in enumerate(places):
            ref, j, r = h_place(i, hs, (2 * u + c // 3) * US)
            ref[j, n, pl.ds(r, US), :] = hb[k * US:(k + 1) * US]

    def flush(acc):
        for n, v in enumerate(acc):
            if v is not None:
                cols = pl.ds(((n % 3) * G + n // 3) * 128, 128)
                ssq[:, cols] = v + ssq[:, cols]

    NU = TM // (2 * US)
    NS = NU * G // NL
    assert NU * G % NL == 0 and NS % G == 0

    def live_at(t):
        return [u for u in range(1 - NL, NU) if 0 <= t - (G * u) // NL < G]

    assert 2 * US * min(live_at(NS - 1)) >= TH and TC >= 128
    deferred = [c for c, _ in block_products(ORDER1, lambda r: 0.0)][6 - ND:]

    def activate_deferred(i, acc):
        for k, c in enumerate(deferred):
            activate(ybuf[k], [(i, None, u) for u in live_at(NS - 1)], c, G - 1, acc)

    def pass1(step, hs):
        i = NB - 1 - step

        @pl.when(i >= NX - 1)
        def _():
            x_in(i - (NX - 1)).start()

        @pl.when(i >= 1)
        def _():
            x_in(i - 1).wait()

        @pl.when(i + NH < NB)
        def _():
            h_out(i + NH, hs).wait()

        acc = [None] * NT
        prev = jnp.minimum(i + 1, NB - 1)
        activate_deferred(prev, acc)
        units = {k - (NL - 1): [fbuf[k, r] for r in range(15)] for k in range(NL)}
        for t in range(NS):
            for u in (live_at(t + 1) if t + 1 < NS else [NU]):
                if u not in units:
                    units[u] = left_unit(x_slot(i), u) if u < NU else left_unit(x_slot(jnp.maximum(i - 1, 0)), 0)
            live = live_at(t)
            for c, y in first_matmul([units[u] for u in live], lambda r: weight(r, t % G)):
                if t == NS - 1 and c in deferred:
                    ybuf[deferred.index(c)] = y
                else:
                    activate(y, [(i, hs, u) if u >= 0 else (prev, None, u + NU) for u in live], c, t % G, acc)
        for k in range(NL):
            for r in range(15):
                fbuf[k, r] = units[NU - (NL - 1) + k][r].astype(BF16)
        flush(acc)

        @pl.when(i >= NH)
        def _():
            h_out(i, hs).start()

        return jnp.where(hs == 0, NH - 1, hs - 1)

    w1_in = [pltpu.make_async_copy(w1_hbm.at[pl.ds(k * 128, 128), pl.ds(n * 128, 128)],
                                   hcache.at[k, n, pl.ds(0, 128)], sem_w.at[0])
             for k in range(3) for n in range(NT)]
    w1_in.append(pltpu.make_async_copy(dw_hbm, dw_ref, sem_w.at[0]))
    w2_in = [pltpu.make_async_copy(w2_hbm.at[:, pl.ds(n * 128, 128)], aux.at[n], sem_w.at[1]) for n in range(3)]
    for cp in w1_in:
        cp.start()
    ssq[...] = jnp.zeros_like(ssq)
    ybuf[...] = jnp.zeros_like(ybuf)
    fbuf[...] = jnp.zeros_like(fbuf)
    for cp in w1_in:
        cp.wait()
    x_in(NB - 1).start()
    for q in range(G):
        blocks = [hcache[j // 3, (j % 3) * G + q, pl.ds(0, 128), :].astype(F32) for j in range(9)]
        for r in range(15):
            wc[r, q] = pltpu.bitcast(signed_sum(B_FORMS[r], blocks.__getitem__).astype(BF16), U32)
    x_in(NB - 1).wait()
    for s in range(1, NX - 1):
        x_in(NB - 1 - s).start()
    for cp in w2_in:
        cp.start()
    for r, f in enumerate(left_unit(x_slot(NB - 1), 0)):
        fbuf[NL - 1, r] = f.astype(BF16)

    jax.lax.fori_loop(0, NB, pass1, jnp.int32((NB - 1) % NH))

    acc = [None] * NT
    activate_deferred(0, acc)
    for t in range(G - 1):
        live = [u for u in live_at(t) if u < 0]
        if live:
            carried = [[fbuf[u + NL - 1, r] for r in range(15)] for u in live]
            for c, y in first_matmul(carried, lambda r: weight(r, t)):
                activate(y, [(0, None, NU + u) for u in live], c, t, acc)
    flush(acc)

    for cp in w2_in:
        cp.wait()
    gx = jnp.sqrt(jnp.sum(ssq[...], axis=0, keepdims=True) * (HSCALE * HSCALE) + 1e-6)
    nx = gx / (jnp.mean(gx, axis=-1, keepdims=True) + 1e-6)
    scale = (1.0 + g_ref[...].astype(F32).reshape(1, D) * nx) * HSCALE
    b_rows = jnp.broadcast_to(b_ref[...].astype(F32).reshape(1, D), (16, D)).astype(BF16)
    bias = jnp.dot(b_rows, jnp.concatenate([aux[n] for n in range(3)], axis=1), preferred_element_type=F32)[0:1]
    for q in range(G):
        col = [jnp.broadcast_to(scale[:, (k * G + q) * 128:(k * G + q + 1) * 128], (128, 128)).T for k in range(3)]
        blocks = [aux[j % 3, pl.ds(((j // 3) * G + q) * 128, 128), :].astype(F32) * col[j // 3] for j in range(9)]
        for r in range(15):
            if q == G - 1:
                aux[r // NT, pl.ds((r % NT) * 128, 128), :] = weight(r, q)
            wc[r, q] = pltpu.bitcast(signed_sum(B_FORMS[r], blocks.__getitem__).astype(BF16), U32)

    def pass2(i, hs):
        @pl.when(i >= 2)
        def _():
            o_out(i - 2).wait()

        @pl.when(jnp.logical_and(i >= 2, i + NX - 2 < NB))
        def _():
            x_in(i + NX - 2).start()

        @pl.when(i >= NH)
        def _():
            for cp in h_in(i, hs):
                cp.wait()

        @pl.when(i >= NX)
        def _():
            x_in(i).wait()

        for r0 in range(0, TM, 2 * M2):
            if r0 == RP:
                redo = range((TH - RR) // (2 * US), TH // (2 * US))
                for c, y in first_matmul([left_unit(x_slot(i), u) for u in redo],
                                         lambda r: aux[r // NT, pl.ds((r % NT) * 128, 128), :]):
                    activate(y, [(i, hs, u) for u in redo], c, G - 1, None)
            if r0 == TH:
                @pl.when(i + NH < NB)
                def _():
                    for cp in h_in(i + NH, hs):
                        cp.start()

            raw = []
            for half in range(2):
                ref, j, r = h_place(i, hs, r0 + half * M2)
                raw += [jnp.concatenate([ref[j, 3 * q + k, pl.ds(r, M2), :] for q in range(G)], axis=1)
                        for k in range(3)]
            forms = a_forms([v.astype(F32) for v in raw])
            forms = [raw[4], raw[1], raw[2], raw[3]] + [f.astype(BF16) for f in forms[4:]]

            def product(r):
                rhs = jnp.concatenate([weight(r, q) for q in range(G)], axis=0)
                return jnp.dot(forms[r], rhs, preferred_element_type=F32)

            for c, y in block_products(ORDER2, product):
                rows = pl.ds(r0 + (c // 3) * M2, M2)
                cols = slice((c % 3) * 128, (c % 3 + 1) * 128)
                residual = xbuf[x_slot(i), rows, cols].astype(F32)
                xbuf[x_slot(i), rows, cols] = (y + bias[:, cols] + residual).astype(BF16)
        o_out(i).start()
        return jnp.where(hs == NH - 1, 0, hs + 1)

    assert TH % (2 * M2) == 0 and RP % (2 * M2) == 0 and RP < TH - RR and RR % (2 * US) == 0
    jax.lax.fori_loop(0, NB, pass2, jnp.int32(0))
    o_out(NB - 2).wait()
    o_out(NB - 1).wait()


@jax.jit
def pallas_standalone__modern_conv_block_slak__vision_kernel(
    x: jax.Array,
    dw: jax.Array,
    w1: jax.Array,
    w2: jax.Array,
    grn_g: jax.Array,
    grn_b: jax.Array,
):
    B, H, W, C = x.shape
    N = B * H * W
    D = w1.shape[1]
    NB = N // TM
    NT = D // 128
    assert B == 1 and dw.shape[:2] == (1, 1) and C == 384 and D == 4 * C and N % TM == 0 and NB > NX
    assert all(a.dtype == BF16 for a in (x, dw, w1, w2))
    hbm = pl.BlockSpec(memory_space=pl.ANY)
    vmem = pl.BlockSpec(memory_space=pltpu.VMEM)
    out, _ = pl.pallas_call(
        _kernel,
        in_specs=[hbm, hbm, hbm, hbm, vmem, vmem],
        out_specs=[hbm, hbm],
        out_shape=[
            jax.ShapeDtypeStruct((N, C), x.dtype),
            jax.ShapeDtypeStruct((NB - NH, NT, TH, 128), BF16),
        ],
        scratch_shapes=[
            pltpu.VMEM((NX, TM, C), BF16),
            pltpu.VMEM((NH, NT, TH, 128), BF16),
            pltpu.VMEM((NB, NT, TC, 128), BF16),
            pltpu.VMEM((15, NT // 3, 64, 128), U32),
            pltpu.VMEM((NL, 15, US, 128), BF16),
            pltpu.VMEM((ND, NL * US, 128), F32),
            pltpu.VMEM((8, D), F32),
            pltpu.VMEM((1, C), BF16),
            pltpu.VMEM((3, D, 128), BF16),
            pltpu.SemaphoreType.DMA((NX,)),
            pltpu.SemaphoreType.DMA((NH,)),
            pltpu.SemaphoreType.DMA((2,)),
        ],
        compiler_params=pltpu.CompilerParams(
            vmem_limit_bytes=128 * 1024 * 1024, disable_bounds_checks=True),
    )(x.reshape(N, C), dw.reshape(1, C), w1, w2, grn_g, grn_b)
    return out.reshape(x.shape)
```

```python
import numpy as np
import jax
import jax.numpy as jnp
import jax.experimental.pallas as pl
import jax.experimental.pallas.tpu as pltpu

F32 = jnp.float32
BF16 = jnp.bfloat16
U32 = jnp.uint32

_C0 = float(np.sqrt(2.0 / np.pi))
ALPHA = float((_C0 * 0.044715) ** (1.0 / 3.0))
BETA = _C0 / ALPHA
HSCALE = 0.5 / ALPHA

TM = 1536
TC = 384
TH = TM - TC
NH = 3
NX = 4
US = 16
NL = 3
ND = 3
M2 = 32
RR = 128
RP = 64

B_FORMS = (
    (0, 0, 0, -1, 1, 0, -1, 0, 0),
    (-1, 0, 0, -1, 0, 1, 0, 0, 0),
    (0, 0, -1, 0, 0, 0, -1, 0, 1),
    (1, -1, 0, 0, 0, 0, 0, 1, 0),
    (0, 0, 0, 0, 0, -1, 0, -1, -1),
    (0, -1, -1, 0, -1, 0, 0, 0, 0),
    (0, 0, 1, 0, 0, 0, 0, 0, 0),
    (0, 0, 0, 0, 0, 0, 0, -1, 0),
    (0, 0, -1, 0, 0, 0, 0, -1, 0),
    (-1, 0, 0, 0, 0, 0, 0, 0, 0),
    (0, 0, 0, 0, 0, 0, -1, 0, 0),
    (1, 0, 0, 0, 1, 0, 0, 0, 0),
    (0, 0, 0, 0, 0, 1, 1, 0, 0),
    (0, 0, 0, 0, -1, 0, 0, 0, 0),
    (0, 0, 0, 0, 0, -1, 0, 0, 0),
)


def a_forms(a):
    a0, a1, a2, a3, a4, a5 = a
    d54 = a5 - a4
    d10 = a1 - a0
    e = a3 - d10
    f = d54 + a2
    return [a4, a1, a2, a3, a2 + a5, a0 + a3, a0 + a2, a3 + a5, a3 - a2, d10, d54, e, f, a4 - e, a1 - f]


C_SUMS = {
    "t1": {"p10": 1, "p12": 1},
    "t2": {"t1": 1, "p14": -1},
    "t3": {"p11": 1, "p9": -1},
    "t4": {"t3": 1, "p13": -1},
    "c0": {"t2": 1, "p9": 1, "p1": -1},
    "c1": {"p3": 1, "t3": -1, "p6": -1, "p8": 1, "p5": -1},
    "c2": {"t2": 1, "p2": 1, "p6": 1},
    "c3": {"t4": 1, "p10": -1, "p0": -1},
    "c4": {"t4": 1, "p3": -1, "p7": -1},
    "c5": {"p7": 1, "t1": -1, "p2": -1, "p8": -1, "p4": -1},
}

ORDER1 = (10, 12, 14, 9, 1, 11, 13, 0, 2, 6, 3, 7, 4, 8, 5)
ORDER2 = (1, 2, 3, 0, 10, 12, 14, 9, 6, 11, 13, 7, 8, 4, 5)


def block_products(order, product):
    partial = {name: None for name in C_SUMS}
    missing = {name: len(terms) for name, terms in C_SUMS.items()}
    for r in order:
        arrived = [("p%d" % r, product(r))]
        while arrived:
            term, v = arrived.pop(0)
            for name, terms in C_SUMS.items():
                if term not in terms:
                    continue
                sign = terms[term]
                if partial[name] is None:
                    partial[name] = (sign, v)
                else:
                    s0, v0 = partial[name]
                    partial[name] = (s0, v0 + v) if s0 == sign else (1, v0 - v if s0 > 0 else v - v0)
                missing[name] -= 1
                if missing[name] == 0:
                    assert partial[name][0] > 0
                    if name[0] == "t":
                        arrived.append((name, partial[name][1]))
                    else:
                        yield int(name[1]), partial[name][1]


def signed_sum(coefs, get):
    acc = None
    for j, c in enumerate(coefs):
        if c:
            v = get(j)
            acc = (v if c > 0 else -v) if acc is None else (acc + v if c > 0 else acc - v)
    return acc


def _kernel(x_hbm, dw_hbm, w1_hbm, w2_hbm, g_ref, b_ref, o_hbm, h_hbm,
            xbuf, hbuf, hcache, wc, fbuf, ybuf, ssq, dw_ref, aux, sem_x, sem_h, sem_w):
    N, C = x_hbm.shape
    D = w1_hbm.shape[1]
    NB = N // TM
    NT = D // 128
    G = NT // 3

    def x_slot(i):
        return i & (NX - 1)

    def x_in(i):
        return pltpu.make_async_copy(x_hbm.at[pl.ds(i * TM, TM)], xbuf.at[x_slot(i)], sem_x.at[x_slot(i)])

    def o_out(i):
        return pltpu.make_async_copy(xbuf.at[x_slot(i)], o_hbm.at[pl.ds(i * TM, TM)], sem_x.at[x_slot(i)])

    def h_out(i, hs):
        return pltpu.make_async_copy(hbuf.at[hs], h_hbm.at[i - NH], sem_h.at[hs])

    def h_in(i, hs):
        pieces = ((pl.ds(0, NT - 3),), (pl.ds(NT - 3, 3), pl.ds(0, TH - RR)))
        return [pltpu.make_async_copy(h_hbm.at[(i - NH, *p)], hbuf.at[(hs, *p)], sem_h.at[hs]) for p in pieces]

    def h_place(i, hs, r0):
        return (hcache, i, r0 - TH) if r0 >= TH else (hbuf, hs, r0)

    def weight(r, q):
        return pltpu.bitcast(wc[r, q], BF16)

    def left_unit(slot, u):
        dw = dw_ref[...].astype(F32)
        groups = range(0, US, 8)
        xc, ss = [], []
        for r0 in [(2 * u + half) * US + k for k in groups for half in range(2)]:
            xv = xbuf[slot, pl.ds(r0, 8), :].astype(F32) * dw
            xc.append(xv - jnp.sum(xv, axis=-1, keepdims=True) * (1.0 / C))
            ss.append(jnp.sum(xc[-1] * xc[-1], axis=-1, keepdims=True))
        a = [v * jax.lax.rsqrt(t * (1.0 / (C * ALPHA * ALPHA)) + 1e-5 / (ALPHA * ALPHA)) for v, t in zip(xc, ss)]
        forms = [a_forms([v[:, k * 128:(k + 1) * 128] for v in a[2 * g:2 * g + 2] for k in range(3)])
                 for g in range(len(groups))]
        return [jnp.concatenate([f[r] for f in forms], axis=0) for r in range(15)]

    def first_matmul(units, rhs):
        def product(r):
            fresh = [u[r] for u in units if u[r].dtype == F32]
            lhs = [u[r] for u in units if u[r].dtype == BF16]
            if fresh:
                lhs.append(jnp.concatenate(fresh, axis=0).astype(BF16))
            return jnp.dot(jnp.concatenate(lhs, axis=0), rhs(r), preferred_element_type=F32)
        return block_products(ORDER1, product)

    def activate(y, places, c, q, acc):
        n = 3 * q + c % 3
        h = y * (1.0 + jnp.tanh(y * (y * y + BETA)))
        if acc is not None:
            sq = h * h
            for k in range(0, y.shape[0], 16):
                pair = sq[k:k + 8] + sq[k + 8:k + 16]
                acc[n] = pair if acc[n] is None else acc[n] + pair
        hb = h.astype(BF16)
        for k, (i, hs, u) in enumerate(places):
            ref, j, r = h_place(i, hs, (2 * u + c // 3) * US)
            ref[j, n, pl.ds(r, US), :] = hb[k * US:(k + 1) * US]

    def flush(acc):
        for n, v in enumerate(acc):
            if v is not None:
                cols = pl.ds(((n % 3) * G + n // 3) * 128, 128)
                ssq[:, cols] = v + ssq[:, cols]

    NU = TM // (2 * US)
    NS = NU * G // NL
    assert NU * G % NL == 0 and NS % G == 0

    def live_at(t):
        return [u for u in range(1 - NL, NU) if 0 <= t - (G * u) // NL < G]

    assert 2 * US * min(live_at(NS - 1)) >= TH and TC >= 128
    deferred = [c for c, _ in block_products(ORDER1, lambda r: 0.0)][6 - ND:]

    def activate_deferred(i, acc):
        for k, c in enumerate(deferred):
            activate(ybuf[k], [(i, None, u) for u in live_at(NS - 1)], c, G - 1, acc)

    def pass1(step, hs):
        i = NB - 1 - step

        @pl.when(i >= NX - 1)
        def _():
            x_in(i - (NX - 1)).start()

        @pl.when(i >= 1)
        def _():
            x_in(i - 1).wait()

        @pl.when(i + NH < NB)
        def _():
            h_out(i + NH, hs).wait()

        acc = [None] * NT
        prev = jnp.minimum(i + 1, NB - 1)
        activate_deferred(prev, acc)
        units = {k - (NL - 1): [fbuf[k, r] for r in range(15)] for k in range(NL)}
        for t in range(NS):
            for u in (live_at(t + 1) if t + 1 < NS else [NU]):
                if u not in units:
                    units[u] = left_unit(x_slot(i), u) if u < NU else left_unit(x_slot(jnp.maximum(i - 1, 0)), 0)
            live = live_at(t)
            for c, y in first_matmul([units[u] for u in live], lambda r: weight(r, t % G)):
                if t == NS - 1 and c in deferred:
                    ybuf[deferred.index(c)] = y
                else:
                    activate(y, [(i, hs, u) if u >= 0 else (prev, None, u + NU) for u in live], c, t % G, acc)
        for k in range(NL):
            for r in range(15):
                fbuf[k, r] = units[NU - (NL - 1) + k][r].astype(BF16)
        flush(acc)

        @pl.when(i >= NH)
        def _():
            h_out(i, hs).start()

        return jnp.where(hs == 0, NH - 1, hs - 1)

    w1_in = [pltpu.make_async_copy(w1_hbm.at[pl.ds(k * 128, 128), pl.ds(n * 128, 128)],
                                   hcache.at[k, n, pl.ds(0, 128)], sem_w.at[0])
             for k in range(3) for n in range(NT)]
    w1_in.append(pltpu.make_async_copy(dw_hbm, dw_ref, sem_w.at[0]))
    w2_in = [pltpu.make_async_copy(w2_hbm.at[:, pl.ds(n * 128, 128)], aux.at[n], sem_w.at[1]) for n in range(3)]
    for cp in w1_in:
        cp.start()
    ssq[...] = jnp.zeros_like(ssq)
    ybuf[...] = jnp.zeros_like(ybuf)
    fbuf[...] = jnp.zeros_like(fbuf)
    for cp in w1_in:
        cp.wait()
    x_in(NB - 1).start()
    for q in range(G):
        blocks = [hcache[j // 3, (j % 3) * G + q, pl.ds(0, 128), :].astype(F32) for j in range(9)]
        for r in range(15):
            wc[r, q] = pltpu.bitcast(signed_sum(B_FORMS[r], blocks.__getitem__).astype(BF16), U32)
    x_in(NB - 1).wait()
    for s in range(1, NX - 1):
        x_in(NB - 1 - s).start()
    for cp in w2_in:
        cp.start()
    for r, f in enumerate(left_unit(x_slot(NB - 1), 0)):
        fbuf[NL - 1, r] = f.astype(BF16)

    jax.lax.fori_loop(0, NB, pass1, jnp.int32((NB - 1) % NH))

    acc = [None] * NT
    activate_deferred(0, acc)
    for t in range(G - 1):
        live = [u for u in live_at(t) if u < 0]
        if live:
            carried = [[fbuf[u + NL - 1, r] for r in range(15)] for u in live]
            for c, y in first_matmul(carried, lambda r: weight(r, t)):
                activate(y, [(0, None, NU + u) for u in live], c, t, acc)
    flush(acc)

    for cp in w2_in:
        cp.wait()
    gx = jnp.sqrt(jnp.sum(ssq[...], axis=0, keepdims=True) * (HSCALE * HSCALE) + 1e-6)
    nx = gx / (jnp.mean(gx, axis=-1, keepdims=True) + 1e-6)
    scale = (1.0 + g_ref[...].astype(F32).reshape(1, D) * nx) * HSCALE
    b_rows = jnp.broadcast_to(b_ref[...].astype(F32).reshape(1, D), (16, D)).astype(BF16)
    bias = jnp.dot(b_rows, jnp.concatenate([aux[n] for n in range(3)], axis=1), preferred_element_type=F32)[0:1]
    for q in range(G):
        col = [jnp.broadcast_to(scale[:, (k * G + q) * 128:(k * G + q + 1) * 128], (128, 128)).T for k in range(3)]
        blocks = [aux[j % 3, pl.ds(((j // 3) * G + q) * 128, 128), :].astype(F32) * col[j // 3] for j in range(9)]
        for r in range(15):
            if q == G - 1:
                aux[r // NT, pl.ds((r % NT) * 128, 128), :] = weight(r, q)
            wc[r, q] = pltpu.bitcast(signed_sum(B_FORMS[r], blocks.__getitem__).astype(BF16), U32)

    def pass2(i, hs):
        @pl.when(i >= 2)
        def _():
            o_out(i - 2).wait()

        @pl.when(jnp.logical_and(i >= 2, i + NX - 2 < NB))
        def _():
            x_in(i + NX - 2).start()

        @pl.when(i >= NH)
        def _():
            for cp in h_in(i, hs):
                cp.wait()

        @pl.when(i >= NX)
        def _():
            x_in(i).wait()

        for r0 in range(0, TM, 2 * M2):
            if r0 == RP:
                redo = range((TH - RR) // (2 * US), TH // (2 * US))
                for c, y in first_matmul([left_unit(x_slot(i), u) for u in redo],
                                         lambda r: aux[r // NT, pl.ds((r % NT) * 128, 128), :]):
                    activate(y, [(i, hs, u) for u in redo], c, G - 1, None)
            if r0 == TH:
                @pl.when(i + NH < NB)
                def _():
                    for cp in h_in(i + NH, hs):
                        cp.start()

            raw = []
            for half in range(2):
                ref, j, r = h_place(i, hs, r0 + half * M2)
                raw += [jnp.concatenate([ref[j, 3 * q + k, pl.ds(r, M2), :] for q in range(G)], axis=1)
                        for k in range(3)]
            forms = a_forms([v.astype(F32) for v in raw])
            forms = [raw[4], raw[1], raw[2], raw[3]] + [f.astype(BF16) for f in forms[4:]]

            def product(r):
                rhs = jnp.concatenate([weight(r, q) for q in range(G)], axis=0)
                return jnp.dot(forms[r], rhs, preferred_element_type=F32)

            for c, y in block_products(ORDER2, product):
                rows = pl.ds(r0 + (c // 3) * M2, M2)
                cols = slice((c % 3) * 128, (c % 3 + 1) * 128)
                residual = xbuf[x_slot(i), rows, cols].astype(F32)
                xbuf[x_slot(i), rows, cols] = (y + bias[:, cols] + residual).astype(BF16)
        o_out(i).start()
        return jnp.where(hs == NH - 1, 0, hs + 1)

    assert TH % (2 * M2) == 0 and RP % (2 * M2) == 0 and RP < TH - RR and RR % (2 * US) == 0
    jax.lax.fori_loop(0, NB, pass2, jnp.int32(0))
    o_out(NB - 2).wait()
    o_out(NB - 1).wait()


@jax.jit
def pallas_standalone__modern_conv_block_slak__vision_kernel(
    x: jax.Array,
    dw: jax.Array,
    w1: jax.Array,
    w2: jax.Array,
    grn_g: jax.Array,
    grn_b: jax.Array,
):
    B, H, W, C = x.shape
    N = B * H * W
    D = w1.shape[1]
    NB = N // TM
    NT = D // 128
    assert B == 1 and dw.shape[:2] == (1, 1) and C == 384 and D == 4 * C and N % TM == 0 and NB > NX
    assert all(a.dtype == BF16 for a in (x, dw, w1, w2))
    hbm = pl.BlockSpec(memory_space=pl.ANY)
    vmem = pl.BlockSpec(memory_space=pltpu.VMEM)
    out, _ = pl.pallas_call(
        _kernel,
        in_specs=[hbm, hbm, hbm, hbm, vmem, vmem],
        out_specs=[hbm, hbm],
        out_shape=[
            jax.ShapeDtypeStruct((N, C), x.dtype),
            jax.ShapeDtypeStruct((NB - NH, NT, TH, 128), BF16),
        ],
        scratch_shapes=[
            pltpu.VMEM((NX, TM, C), BF16),
            pltpu.VMEM((NH, NT, TH, 128), BF16),
            pltpu.VMEM((NB, NT, TC, 128), BF16),
            pltpu.VMEM((15, NT // 3, 64, 128), U32),
            pltpu.VMEM((NL, 15, US, 128), BF16),
            pltpu.VMEM((ND, NL * US, 128), F32),
            pltpu.VMEM((8, D), F32),
            pltpu.VMEM((1, C), BF16),
            pltpu.VMEM((3, D, 128), BF16),
            pltpu.SemaphoreType.DMA((NX,)),
            pltpu.SemaphoreType.DMA((NH,)),
            pltpu.SemaphoreType.DMA((2,)),
        ],
        compiler_params=pltpu.CompilerParams(
            vmem_limit_bytes=128 * 1024 * 1024, disable_bounds_checks=True),
    )(x.reshape(N, C), dw.reshape(1, C), w1, w2, grn_g, grn_b)
    return out.reshape(x.shape)
```

```python
import numpy as np
import jax
import jax.numpy as jnp
import jax.experimental.pallas as pl
import jax.experimental.pallas.tpu as pltpu

F32 = jnp.float32
BF16 = jnp.bfloat16
U32 = jnp.uint32

_C0 = float(np.sqrt(2.0 / np.pi))
ALPHA = float((_C0 * 0.044715) ** (1.0 / 3.0))
BETA = _C0 / ALPHA
HSCALE = 0.5 / ALPHA

TM = 1536
TC = 384
TH = TM - TC
NH = 3
NX = 4
US = 16
NL = 3
ND = 3
M2 = 32
RR = 128
RP = 256
SP = 832

B_FORMS = (
    (0, 0, 0, -1, 1, 0, -1, 0, 0),
    (-1, 0, 0, -1, 0, 1, 0, 0, 0),
    (0, 0, -1, 0, 0, 0, -1, 0, 1),
    (1, -1, 0, 0, 0, 0, 0, 1, 0),
    (0, 0, 0, 0, 0, -1, 0, -1, -1),
    (0, -1, -1, 0, -1, 0, 0, 0, 0),
    (0, 0, 1, 0, 0, 0, 0, 0, 0),
    (0, 0, 0, 0, 0, 0, 0, -1, 0),
    (0, 0, -1, 0, 0, 0, 0, -1, 0),
    (-1, 0, 0, 0, 0, 0, 0, 0, 0),
    (0, 0, 0, 0, 0, 0, -1, 0, 0),
    (1, 0, 0, 0, 1, 0, 0, 0, 0),
    (0, 0, 0, 0, 0, 1, 1, 0, 0),
    (0, 0, 0, 0, -1, 0, 0, 0, 0),
    (0, 0, 0, 0, 0, -1, 0, 0, 0),
)


def a_forms(a):
    a0, a1, a2, a3, a4, a5 = a
    d54 = a5 - a4
    d10 = a1 - a0
    e = a3 - d10
    f = d54 + a2
    return [a4, a1, a2, a3, a2 + a5, a0 + a3, a0 + a2, a3 + a5, a3 - a2, d10, d54, e, f, a4 - e, a1 - f]


C_SUMS = {
    "t1": {"p10": 1, "p12": 1},
    "t2": {"t1": 1, "p14": -1},
    "t3": {"p11": 1, "p9": -1},
    "t4": {"t3": 1, "p13": -1},
    "c0": {"t2": 1, "p9": 1, "p1": -1},
    "c1": {"p3": 1, "t3": -1, "p6": -1, "p8": 1, "p5": -1},
    "c2": {"t2": 1, "p2": 1, "p6": 1},
    "c3": {"t4": 1, "p10": -1, "p0": -1},
    "c4": {"t4": 1, "p3": -1, "p7": -1},
    "c5": {"p7": 1, "t1": -1, "p2": -1, "p8": -1, "p4": -1},
}

ORDER1 = (10, 12, 14, 9, 1, 2, 6, 11, 13, 0, 3, 7, 8, 4, 5)
ORDER2 = (1, 2, 3, 0, 10, 12, 14, 9, 6, 11, 13, 7, 8, 4, 5)


def block_products(order, product):
    partial = {name: None for name in C_SUMS}
    missing = {name: len(terms) for name, terms in C_SUMS.items()}
    for r in order:
        arrived = [("p%d" % r, product(r))]
        while arrived:
            term, v = arrived.pop(0)
            for name, terms in C_SUMS.items():
                if term not in terms:
                    continue
                sign = terms[term]
                if partial[name] is None:
                    partial[name] = (sign, v)
                else:
                    s0, v0 = partial[name]
                    partial[name] = (s0, v0 + v) if s0 == sign else (1, v0 - v if s0 > 0 else v - v0)
                missing[name] -= 1
                if missing[name] == 0:
                    assert partial[name][0] > 0
                    if name[0] == "t":
                        arrived.append((name, partial[name][1]))
                    else:
                        yield int(name[1]), partial[name][1]


def signed_sum(coefs, get):
    acc = None
    for j, c in enumerate(coefs):
        if c:
            v = get(j)
            acc = (v if c > 0 else -v) if acc is None else (acc + v if c > 0 else acc - v)
    return acc


def _kernel(x_hbm, dw_hbm, w1_hbm, w2_hbm, g_ref, b_ref, o_hbm, h_hbm,
            xbuf, hbuf, hcache, wc, fbuf, ybuf, ssq, dw_ref, aux, sem_x, sem_h, sem_w):
    N, C = x_hbm.shape
    D = w1_hbm.shape[1]
    NB = N // TM
    NT = D // 128
    G = NT // 3

    def x_slot(i):
        return i & (NX - 1)

    def x_in(i):
        return pltpu.make_async_copy(x_hbm.at[pl.ds(i * TM, TM)], xbuf.at[x_slot(i)], sem_x.at[x_slot(i)])

    def o_out(i):
        return pltpu.make_async_copy(xbuf.at[x_slot(i)], o_hbm.at[pl.ds(i * TM, TM)], sem_x.at[x_slot(i)])

    def h_out(i, hs):
        return pltpu.make_async_copy(hbuf.at[hs], h_hbm.at[i - NH], sem_h.at[hs])

    def h_in(i, hs, part):
        if part == 0:
            pieces = [(pl.ds(0, NT), pl.ds(0, SP))]
        else:
            pieces = [(pl.ds(0, NT - 3), pl.ds(SP, TH - SP)), (pl.ds(NT - 3, 3), pl.ds(SP, TH - RR - SP))]
        return [pltpu.make_async_copy(h_hbm.at[(i - NH, *p)], hbuf.at[(hs, *p)], sem_h.at[hs]) for p in pieces]

    def h_place(i, hs, r0):
        return (hcache, i, r0 - TH) if r0 >= TH else (hbuf, hs, r0)

    def weight(r, q):
        return pltpu.bitcast(wc[r, q], BF16)

    def left_unit(slot, u):
        dw = dw_ref[...].astype(F32)
        groups = range(0, US, 8)
        xc, ss = [], []
        for r0 in [(2 * u + half) * US + k for k in groups for half in range(2)]:
            xv = xbuf[slot, pl.ds(r0, 8), :].astype(F32) * dw
            xc.append(xv - jnp.sum(xv, axis=-1, keepdims=True) * (1.0 / C))
            ss.append(jnp.sum(xc[-1] * xc[-1], axis=-1, keepdims=True))
        var = [t * (1.0 / (C * ALPHA * ALPHA)) + 1e-5 / (ALPHA * ALPHA) for t in ss]
        a = [v * jnp.exp2(-0.5 * jnp.log2(t)) for v, t in zip(xc, var)]
        forms = [a_forms([v[:, k * 128:(k + 1) * 128] for v in a[2 * g:2 * g + 2] for k in range(3)])
                 for g in range(len(groups))]
        return [jnp.concatenate([f[r] for f in forms], axis=0) for r in range(15)]

    def first_matmul(units, rhs):
        def product(r):
            fresh = [u[r] for u in units if u[r].dtype == F32]
            lhs = [u[r] for u in units if u[r].dtype == BF16]
            if fresh:
                lhs.append(jnp.concatenate(fresh, axis=0).astype(BF16))
            return jnp.dot(jnp.concatenate(lhs, axis=0), rhs(r), preferred_element_type=F32)
        return block_products(ORDER1, product)

    def activate(y, places, c, q, acc):
        n = 3 * q + c % 3
        h = y * (1.0 + jnp.tanh(y * (y * y + BETA)))
        if acc is not None:
            sq = h * h
            for k in range(0, y.shape[0], 16):
                pair = sq[k:k + 8] + sq[k + 8:k + 16]
                acc[n] = pair if acc[n] is None else acc[n] + pair
        hb = h.astype(BF16)
        for k, (i, hs, u) in enumerate(places):
            ref, j, r = h_place(i, hs, (2 * u + c // 3) * US)
            ref[j, n, pl.ds(r, US), :] = hb[k * US:(k + 1) * US]

    def flush(acc):
        for n, v in enumerate(acc):
            if v is not None:
                cols = pl.ds(((n % 3) * G + n // 3) * 128, 128)
                ssq[:, cols] = v + ssq[:, cols]

    NU = TM // (2 * US)
    NS = NU * G // NL
    assert NU * G % NL == 0 and NS % G == 0

    def live_at(t):
        return [u for u in range(1 - NL, NU) if 0 <= t - (G * u) // NL < G]

    assert 2 * US * min(live_at(NS - 1)) >= TH and TC >= 128
    deferred = [c for c, _ in block_products(ORDER1, lambda r: 0.0)][6 - ND:]

    def activate_deferred(i, acc):
        for k, c in enumerate(deferred):
            activate(ybuf[k], [(i, None, u) for u in live_at(NS - 1)], c, G - 1, acc)

    def pass1(step, hs):
        i = NB - 1 - step

        @pl.when(i >= NX - 1)
        def _():
            x_in(i - (NX - 1)).start()

        @pl.when(i >= 1)
        def _():
            x_in(i - 1).wait()

        @pl.when(i + NH < NB)
        def _():
            h_out(i + NH, hs).wait()

        acc = [None] * NT
        prev = jnp.minimum(i + 1, NB - 1)
        activate_deferred(prev, acc)
        units = {k - (NL - 1): [fbuf[k, r] for r in range(15)] for k in range(NL)}
        for t in range(NS):
            for u in (live_at(t + 1) if t + 1 < NS else [NU]):
                if u not in units:
                    units[u] = left_unit(x_slot(i), u) if u < NU else left_unit(x_slot(jnp.maximum(i - 1, 0)), 0)
            live = live_at(t)
            for c, y in first_matmul([units[u] for u in live], lambda r: weight(r, t % G)):
                if t == NS - 1 and c in deferred:
                    ybuf[deferred.index(c)] = y
                else:
                    activate(y, [(i, hs, u) if u >= 0 else (prev, None, u + NU) for u in live], c, t % G, acc)
        for k in range(NL):
            for r in range(15):
                fbuf[k, r] = units[NU - (NL - 1) + k][r].astype(BF16)
        flush(acc)

        @pl.when(i >= NH)
        def _():
            h_out(i, hs).start()

        return jnp.where(hs == 0, NH - 1, hs - 1)

    w1_in = [pltpu.make_async_copy(w1_hbm.at[pl.ds(k * 128, 128), pl.ds(n * 128, 128)],
                                   hcache.at[k, n, pl.ds(0, 128)], sem_w.at[0])
             for k in range(3) for n in range(NT)]
    w1_in.append(pltpu.make_async_copy(dw_hbm, dw_ref, sem_w.at[0]))
    w2_in = [pltpu.make_async_copy(w2_hbm.at[:, pl.ds(n * 128, 128)], aux.at[n], sem_w.at[1]) for n in range(3)]
    for cp in w1_in:
        cp.start()
    ssq[...] = jnp.zeros_like(ssq)
    ybuf[...] = jnp.zeros_like(ybuf)
    fbuf[...] = jnp.zeros_like(fbuf)
    for cp in w1_in:
        cp.wait()
    x_in(NB - 1).start()
    for q in range(G):
        blocks = [hcache[j // 3, (j % 3) * G + q, pl.ds(0, 128), :].astype(F32) for j in range(9)]
        for r in range(15):
            wc[r, q] = pltpu.bitcast(signed_sum(B_FORMS[r], blocks.__getitem__).astype(BF16), U32)
    x_in(NB - 1).wait()
    for s in range(1, NX - 1):
        x_in(NB - 1 - s).start()
    for cp in w2_in:
        cp.start()
    for r, f in enumerate(left_unit(x_slot(NB - 1), 0)):
        fbuf[NL - 1, r] = f.astype(BF16)

    jax.lax.fori_loop(0, NB, pass1, jnp.int32((NB - 1) % NH))

    acc = [None] * NT
    activate_deferred(0, acc)
    for t in range(G - 1):
        live = [u for u in live_at(t) if u < 0]
        if live:
            carried = [[fbuf[u + NL - 1, r] for r in range(15)] for u in live]
            for c, y in first_matmul(carried, lambda r: weight(r, t)):
                activate(y, [(0, None, NU + u) for u in live], c, t, acc)
    flush(acc)

    for cp in w2_in:
        cp.wait()
    gx = jnp.sqrt(jnp.sum(ssq[...], axis=0, keepdims=True) * (HSCALE * HSCALE) + 1e-6)
    nx = gx / (jnp.mean(gx, axis=-1, keepdims=True) + 1e-6)
    scale = (1.0 + g_ref[...].astype(F32).reshape(1, D) * nx) * HSCALE
    b_rows = jnp.broadcast_to(b_ref[...].astype(F32).reshape(1, D), (16, D)).astype(BF16)
    bias = jnp.dot(b_rows, jnp.concatenate([aux[n] for n in range(3)], axis=1), preferred_element_type=F32)[0:1]
    for q in range(G):
        col = [jnp.broadcast_to(scale[:, (k * G + q) * 128:(k * G + q + 1) * 128], (128, 128)).T for k in range(3)]
        blocks = [aux[j % 3, pl.ds(((j // 3) * G + q) * 128, 128), :].astype(F32) * col[j // 3] for j in range(9)]
        for r in range(15):
            if q == G - 1:
                aux[r // NT, pl.ds((r % NT) * 128, 128), :] = weight(r, q)
            wc[r, q] = pltpu.bitcast(signed_sum(B_FORMS[r], blocks.__getitem__).astype(BF16), U32)

    def pass2(i, hs):
        @pl.when(i >= 2)
        def _():
            o_out(i - 2).wait()

        @pl.when(jnp.logical_and(i >= 2, i + NX - 2 < NB))
        def _():
            x_in(i + NX - 2).start()

        @pl.when(jnp.logical_and(i >= 1, i + NH - 1 < NB))
        def _():
            for cp in h_in(i + NH - 1, jnp.where(hs == 0, NH - 1, hs - 1), 1):
                cp.start()

        @pl.when(i >= NH)
        def _():
            for cp in h_in(i, hs, 0) + h_in(i, hs, 1):
                cp.wait()

        @pl.when(i >= NX)
        def _():
            x_in(i).wait()

        for r0 in range(0, TM, 2 * M2):
            if r0 == RP:
                redo = range((TH - RR) // (2 * US), TH // (2 * US))
                for c, y in first_matmul([left_unit(x_slot(i), u) for u in redo],
                                         lambda r: aux[r // NT, pl.ds((r % NT) * 128, 128), :]):
                    activate(y, [(i, hs, u) for u in redo], c, G - 1, None)
            if r0 == SP:
                @pl.when(i + NH < NB)
                def _():
                    for cp in h_in(i + NH, hs, 0):
                        cp.start()

            raw = []
            for half in range(2):
                ref, j, r = h_place(i, hs, r0 + half * M2)
                raw += [jnp.concatenate([ref[j, 3 * q + k, pl.ds(r, M2), :] for q in range(G)], axis=1)
                        for k in range(3)]
            forms = a_forms([v.astype(F32) for v in raw])
            forms = [raw[4], raw[1], raw[2], raw[3]] + [f.astype(BF16) for f in forms[4:]]

            def product(r):
                rhs = jnp.concatenate([weight(r, q) for q in range(G)], axis=0)
                return jnp.dot(forms[r], rhs, preferred_element_type=F32)

            for c, y in block_products(ORDER2, product):
                rows = pl.ds(r0 + (c // 3) * M2, M2)
                cols = slice((c % 3) * 128, (c % 3 + 1) * 128)
                residual = xbuf[x_slot(i), rows, cols].astype(F32)
                xbuf[x_slot(i), rows, cols] = (y + bias[:, cols] + residual).astype(BF16)
        o_out(i).start()
        return jnp.where(hs == NH - 1, 0, hs + 1)

    assert TH % (2 * M2) == 0 and RP % (2 * M2) == 0 and SP % (2 * M2) == 0 and SP < TH - RR and RP < TH - RR and RR % (2 * US) == 0
    jax.lax.fori_loop(0, NB, pass2, jnp.int32(0))
    o_out(NB - 2).wait()
    o_out(NB - 1).wait()


@jax.jit
def pallas_standalone__modern_conv_block_slak__vision_kernel(
    x: jax.Array,
    dw: jax.Array,
    w1: jax.Array,
    w2: jax.Array,
    grn_g: jax.Array,
    grn_b: jax.Array,
):
    B, H, W, C = x.shape
    N = B * H * W
    D = w1.shape[1]
    NB = N // TM
    NT = D // 128
    assert B == 1 and dw.shape[:2] == (1, 1) and C == 384 and D == 4 * C and N % TM == 0 and NB > NX
    assert all(a.dtype == BF16 for a in (x, dw, w1, w2))
    hbm = pl.BlockSpec(memory_space=pl.ANY)
    vmem = pl.BlockSpec(memory_space=pltpu.VMEM)
    out, _ = pl.pallas_call(
        _kernel,
        in_specs=[hbm, hbm, hbm, hbm, vmem, vmem],
        out_specs=[hbm, hbm],
        out_shape=[
            jax.ShapeDtypeStruct((N, C), x.dtype),
            jax.ShapeDtypeStruct((NB - NH, NT, TH, 128), BF16),
        ],
        scratch_shapes=[
            pltpu.VMEM((NX, TM, C), BF16),
            pltpu.VMEM((NH, NT, TH, 128), BF16),
            pltpu.VMEM((NB, NT, TC, 128), BF16),
            pltpu.VMEM((15, NT // 3, 64, 128), U32),
            pltpu.VMEM((NL, 15, US, 128), BF16),
            pltpu.VMEM((ND, NL * US, 128), F32),
            pltpu.VMEM((8, D), F32),
            pltpu.VMEM((1, C), BF16),
            pltpu.VMEM((3, D, 128), BF16),
            pltpu.SemaphoreType.DMA((NX,)),
            pltpu.SemaphoreType.DMA((NH,)),
            pltpu.SemaphoreType.DMA((2,)),
        ],
        compiler_params=pltpu.CompilerParams(
            vmem_limit_bytes=128 * 1024 * 1024, disable_bounds_checks=True),
    )(x.reshape(N, C), dw.reshape(1, C), w1, w2, grn_g, grn_b)
    return out.reshape(x.shape)
```

```python
import numpy as np
import jax
import jax.numpy as jnp
import jax.experimental.pallas as pl
import jax.experimental.pallas.tpu as pltpu

F32 = jnp.float32
BF16 = jnp.bfloat16
U32 = jnp.uint32

_C0 = float(np.sqrt(2.0 / np.pi))
ALPHA = float((_C0 * 0.044715) ** (1.0 / 3.0))
BETA = _C0 / ALPHA
HSCALE = 0.5 / ALPHA

TM = 1536
TC = 384
TH = TM - TC
NH = 3
NX = 4
US = 16
NL = 3
ND = 3
M2 = 32
RR = 128
RP = 576
SP = 832

B_FORMS = (
    (0, 0, 0, -1, 1, 0, -1, 0, 0),
    (-1, 0, 0, -1, 0, 1, 0, 0, 0),
    (0, 0, -1, 0, 0, 0, -1, 0, 1),
    (1, -1, 0, 0, 0, 0, 0, 1, 0),
    (0, 0, 0, 0, 0, -1, 0, -1, -1),
    (0, -1, -1, 0, -1, 0, 0, 0, 0),
    (0, 0, 1, 0, 0, 0, 0, 0, 0),
    (0, 0, 0, 0, 0, 0, 0, -1, 0),
    (0, 0, -1, 0, 0, 0, 0, -1, 0),
    (-1, 0, 0, 0, 0, 0, 0, 0, 0),
    (0, 0, 0, 0, 0, 0, -1, 0, 0),
    (1, 0, 0, 0, 1, 0, 0, 0, 0),
    (0, 0, 0, 0, 0, 1, 1, 0, 0),
    (0, 0, 0, 0, -1, 0, 0, 0, 0),
    (0, 0, 0, 0, 0, -1, 0, 0, 0),
)


def a_forms(a):
    a0, a1, a2, a3, a4, a5 = a
    d54 = a5 - a4
    d10 = a1 - a0
    e = a3 - d10
    f = d54 + a2
    return [a4, a1, a2, a3, a2 + a5, a0 + a3, a0 + a2, a3 + a5, a3 - a2, d10, d54, e, f, a4 - e, a1 - f]


C_SUMS = {
    "t1": {"p10": 1, "p12": 1},
    "t2": {"t1": 1, "p14": -1},
    "t3": {"p11": 1, "p9": -1},
    "t4": {"t3": 1, "p13": -1},
    "c0": {"t2": 1, "p9": 1, "p1": -1},
    "c1": {"p3": 1, "t3": -1, "p6": -1, "p8": 1, "p5": -1},
    "c2": {"t2": 1, "p2": 1, "p6": 1},
    "c3": {"t4": 1, "p10": -1, "p0": -1},
    "c4": {"t4": 1, "p3": -1, "p7": -1},
    "c5": {"p7": 1, "t1": -1, "p2": -1, "p8": -1, "p4": -1},
}

ORDER1 = (10, 12, 14, 9, 1, 2, 6, 11, 13, 0, 3, 7, 8, 4, 5)
ORDER2 = (1, 2, 3, 0, 10, 12, 14, 9, 6, 11, 13, 7, 8, 4, 5)


def block_products(order, product):
    partial = {name: None for name in C_SUMS}
    missing = {name: len(terms) for name, terms in C_SUMS.items()}
    for r in order:
        arrived = [("p%d" % r, product(r))]
        while arrived:
            term, v = arrived.pop(0)
            for name, terms in C_SUMS.items():
                if term not in terms:
                    continue
                sign = terms[term]
                if partial[name] is None:
                    partial[name] = (sign, v)
                else:
                    s0, v0 = partial[name]
                    partial[name] = (s0, v0 + v) if s0 == sign else (1, v0 - v if s0 > 0 else v - v0)
                missing[name] -= 1
                if missing[name] == 0:
                    assert partial[name][0] > 0
                    if name[0] == "t":
                        arrived.append((name, partial[name][1]))
                    else:
                        yield int(name[1]), partial[name][1]


def signed_sum(coefs, get):
    acc = None
    for j, c in enumerate(coefs):
        if c:
            v = get(j)
            acc = (v if c > 0 else -v) if acc is None else (acc + v if c > 0 else acc - v)
    return acc


def _kernel(x_hbm, dw_hbm, w1_hbm, w2_hbm, g_ref, b_ref, o_hbm, h_hbm,
            xbuf, hbuf, hcache, wc, fbuf, ybuf, ssq, dw_ref, dw_rows, aux, sem_x, sem_h, sem_w):
    N, C = x_hbm.shape
    D = w1_hbm.shape[1]
    NB = N // TM
    NT = D // 128
    G = NT // 3

    def x_slot(i):
        return i & (NX - 1)

    def x_in(i):
        return pltpu.make_async_copy(x_hbm.at[pl.ds(i * TM, TM)], xbuf.at[x_slot(i)], sem_x.at[x_slot(i)])

    def o_out(i):
        return pltpu.make_async_copy(xbuf.at[x_slot(i)], o_hbm.at[pl.ds(i * TM, TM)], sem_x.at[x_slot(i)])

    def h_out(i, hs):
        return pltpu.make_async_copy(hbuf.at[hs], h_hbm.at[i - NH], sem_h.at[hs])

    def h_in(i, hs, part):
        if part == 0:
            pieces = [(pl.ds(0, NT), pl.ds(0, SP))]
        else:
            pieces = [(pl.ds(0, NT - 3), pl.ds(SP, TH - SP)), (pl.ds(NT - 3, 3), pl.ds(SP, TH - RR - SP))]
        return [pltpu.make_async_copy(h_hbm.at[(i - NH, *p)], hbuf.at[(hs, *p)], sem_h.at[hs]) for p in pieces]

    def h_place(i, hs, r0):
        return (hcache, i, r0 - TH) if r0 >= TH else (hbuf, hs, r0)

    def weight(r, q):
        return pltpu.bitcast(wc[r, q], BF16)

    def left_unit(slot, u):
        groups = range(0, US, 8)
        xc, ss = [], []
        for r0 in [(2 * u + half) * US + k for k in groups for half in range(2)]:
            xv = xbuf[slot, pl.ds(r0, 8), :].astype(F32) * dw_rows[...]
            xc.append(xv - jnp.sum(xv, axis=-1, keepdims=True) * (1.0 / C))
            ss.append(jnp.sum(xc[-1] * xc[-1], axis=-1, keepdims=True))
        var = [t * (1.0 / (C * ALPHA * ALPHA)) + 1e-5 / (ALPHA * ALPHA) for t in ss]
        a = [v * jnp.exp2(-0.5 * jnp.log2(t)) for v, t in zip(xc, var)]
        forms = [a_forms([v[:, k * 128:(k + 1) * 128] for v in a[2 * g:2 * g + 2] for k in range(3)])
                 for g in range(len(groups))]
        return [jnp.concatenate([f[r] for f in forms], axis=0) for r in range(15)]

    def first_matmul(units, rhs):
        def product(r):
            fresh = [u[r] for u in units if u[r].dtype == F32]
            lhs = [u[r] for u in units if u[r].dtype == BF16]
            if fresh:
                lhs.append(jnp.concatenate(fresh, axis=0).astype(BF16))
            return jnp.dot(jnp.concatenate(lhs, axis=0), rhs(r), preferred_element_type=F32)
        return block_products(ORDER1, product)

    def activate(y, places, c, q, acc):
        n = 3 * q + c % 3
        h = y * (1.0 + jnp.tanh(y * (y * y + BETA)))
        if acc is not None:
            sq = h * h
            for k in range(0, y.shape[0], 16):
                pair = sq[k:k + 8] + sq[k + 8:k + 16]
                acc[n] = pair if acc[n] is None else acc[n] + pair
        hb = h.astype(BF16)
        for k, (i, hs, u) in enumerate(places):
            ref, j, r = h_place(i, hs, (2 * u + c // 3) * US)
            ref[j, n, pl.ds(r, US), :] = hb[k * US:(k + 1) * US]

    def flush(acc):
        for n, v in enumerate(acc):
            if v is not None:
                cols = pl.ds(((n % 3) * G + n // 3) * 128, 128)
                ssq[:, cols] = v + ssq[:, cols]

    NU = TM // (2 * US)
    NS = NU * G // NL
    assert NU * G % NL == 0 and NS % G == 0

    def live_at(t):
        return [u for u in range(1 - NL, NU) if 0 <= t - (G * u) // NL < G]

    assert 2 * US * min(live_at(NS - 1)) >= TH and TC >= 128
    deferred = [c for c, _ in block_products(ORDER1, lambda r: 0.0)][6 - ND:]

    def activate_deferred(i, acc):
        for k, c in enumerate(deferred):
            activate(ybuf[k], [(i, None, u) for u in live_at(NS - 1)], c, G - 1, acc)

    def pass1(step, hs):
        i = NB - 1 - step

        @pl.when(i >= NX - 1)
        def _():
            x_in(i - (NX - 1)).start()

        @pl.when(i >= 1)
        def _():
            x_in(i - 1).wait()

        @pl.when(i + NH < NB)
        def _():
            h_out(i + NH, hs).wait()

        acc = [None] * NT
        prev = jnp.minimum(i + 1, NB - 1)
        activate_deferred(prev, acc)
        units = {k - (NL - 1): [fbuf[k, r] for r in range(15)] for k in range(NL)}
        for t in range(NS):
            for u in (live_at(t + 1) if t + 1 < NS else [NU]):
                if u not in units:
                    units[u] = left_unit(x_slot(i), u) if u < NU else left_unit(x_slot(jnp.maximum(i - 1, 0)), 0)
            live = live_at(t)
            for c, y in first_matmul([units[u] for u in live], lambda r: weight(r, t % G)):
                if t == NS - 1 and c in deferred:
                    ybuf[deferred.index(c)] = y
                else:
                    activate(y, [(i, hs, u) if u >= 0 else (prev, None, u + NU) for u in live], c, t % G, acc)
        for k in range(NL):
            for r in range(15):
                fbuf[k, r] = units[NU - (NL - 1) + k][r].astype(BF16)
        flush(acc)

        @pl.when(i >= NH)
        def _():
            h_out(i, hs).start()

        return jnp.where(hs == 0, NH - 1, hs - 1)

    w1_in = [pltpu.make_async_copy(w1_hbm.at[pl.ds(k * 128, 128), pl.ds(n * 128, 128)],
                                   hcache.at[k, n, pl.ds(0, 128)], sem_w.at[0])
             for k in range(3) for n in range(NT)]
    w1_in.append(pltpu.make_async_copy(dw_hbm, dw_ref, sem_w.at[0]))
    w2_in = [pltpu.make_async_copy(w2_hbm.at[:, pl.ds(n * 128, 128)], aux.at[n], sem_w.at[1]) for n in range(3)]
    for cp in w1_in:
        cp.start()
    ssq[...] = jnp.zeros_like(ssq)
    ybuf[...] = jnp.zeros_like(ybuf)
    fbuf[...] = jnp.zeros_like(fbuf)
    for cp in w1_in:
        cp.wait()
    x_in(NB - 1).start()
    dw_rows[...] = jnp.broadcast_to(dw_ref[...].astype(F32), (8, C))
    for q in range(G):
        blocks = [hcache[j // 3, (j % 3) * G + q, pl.ds(0, 128), :].astype(F32) for j in range(9)]
        for r in range(15):
            wc[r, q] = pltpu.bitcast(signed_sum(B_FORMS[r], blocks.__getitem__).astype(BF16), U32)
    x_in(NB - 1).wait()
    for s in range(1, NX - 1):
        x_in(NB - 1 - s).start()
    for cp in w2_in:
        cp.start()
    for r, f in enumerate(left_unit(x_slot(NB - 1), 0)):
        fbuf[NL - 1, r] = f.astype(BF16)

    jax.lax.fori_loop(0, NB, pass1, jnp.int32((NB - 1) % NH))

    acc = [None] * NT
    activate_deferred(0, acc)
    for t in range(G - 1):
        live = [u for u in live_at(t) if u < 0]
        if live:
            carried = [[fbuf[u + NL - 1, r] for r in range(15)] for u in live]
            for c, y in first_matmul(carried, lambda r: weight(r, t)):
                activate(y, [(0, None, NU + u) for u in live], c, t, acc)
    flush(acc)

    for cp in w2_in:
        cp.wait()
    gx = jnp.sqrt(jnp.sum(ssq[...], axis=0, keepdims=True) * (HSCALE * HSCALE) + 1e-6)
    nx = gx / (jnp.mean(gx, axis=-1, keepdims=True) + 1e-6)
    scale = (1.0 + g_ref[...].astype(F32).reshape(1, D) * nx) * HSCALE
    b_rows = jnp.broadcast_to(b_ref[...].astype(F32).reshape(1, D), (16, D)).astype(BF16)
    bias = jnp.dot(b_rows, jnp.concatenate([aux[n] for n in range(3)], axis=1), preferred_element_type=F32)[0:1]
    for q in range(G):
        col = [jnp.broadcast_to(scale[:, (k * G + q) * 128:(k * G + q + 1) * 128], (128, 128)).T for k in range(3)]
        blocks = [aux[j % 3, pl.ds(((j // 3) * G + q) * 128, 128), :].astype(F32) * col[j // 3] for j in range(9)]
        for r in range(15):
            if q == G - 1:
                aux[r // NT, pl.ds((r % NT) * 128, 128), :] = weight(r, q)
            wc[r, q] = pltpu.bitcast(signed_sum(B_FORMS[r], blocks.__getitem__).astype(BF16), U32)

    def pass2(i, hs):
        @pl.when(i >= 2)
        def _():
            o_out(i - 2).wait()

        @pl.when(jnp.logical_and(i >= 2, i + NX - 2 < NB))
        def _():
            x_in(i + NX - 2).start()

        @pl.when(jnp.logical_and(i >= 1, i + NH - 1 < NB))
        def _():
            for cp in h_in(i + NH - 1, jnp.where(hs == 0, NH - 1, hs - 1), 1):
                cp.start()

        @pl.when(i >= NH)
        def _():
            for cp in h_in(i, hs, 0) + h_in(i, hs, 1):
                cp.wait()

        @pl.when(i >= NX)
        def _():
            x_in(i).wait()

        for r0 in range(0, TM, 2 * M2):
            if r0 == RP:
                redo = range((TH - RR) // (2 * US), TH // (2 * US))
                for c, y in first_matmul([left_unit(x_slot(i), u) for u in redo],
                                         lambda r: aux[r // NT, pl.ds((r % NT) * 128, 128), :]):
                    activate(y, [(i, hs, u) for u in redo], c, G - 1, None)
            if r0 == SP:
                @pl.when(i + NH < NB)
                def _():
                    for cp in h_in(i + NH, hs, 0):
                        cp.start()

            raw = []
            for half in range(2):
                ref, j, r = h_place(i, hs, r0 + half * M2)
                raw += [jnp.concatenate([ref[j, 3 * q + k, pl.ds(r, M2), :] for q in range(G)], axis=1)
                        for k in range(3)]
            forms = a_forms([v.astype(F32) for v in raw])
            forms = [raw[4], raw[1], raw[2], raw[3]] + [f.astype(BF16) for f in forms[4:]]

            def product(r):
                rhs = jnp.concatenate([weight(r, q) for q in range(G)], axis=0)
                return jnp.dot(forms[r], rhs, preferred_element_type=F32)

            for c, y in block_products(ORDER2, product):
                rows = pl.ds(r0 + (c // 3) * M2, M2)
                cols = slice((c % 3) * 128, (c % 3 + 1) * 128)
                residual = xbuf[x_slot(i), rows, cols].astype(F32)
                xbuf[x_slot(i), rows, cols] = (y + bias[:, cols] + residual).astype(BF16)
        o_out(i).start()
        return jnp.where(hs == NH - 1, 0, hs + 1)

    assert TH % (2 * M2) == 0 and RP % (2 * M2) == 0 and SP % (2 * M2) == 0 and SP < TH - RR and RP < TH - RR and RR % (2 * US) == 0
    jax.lax.fori_loop(0, NB, pass2, jnp.int32(0))
    o_out(NB - 2).wait()
    o_out(NB - 1).wait()


@jax.jit
def pallas_standalone__modern_conv_block_slak__vision_kernel(
    x: jax.Array,
    dw: jax.Array,
    w1: jax.Array,
    w2: jax.Array,
    grn_g: jax.Array,
    grn_b: jax.Array,
):
    B, H, W, C = x.shape
    N = B * H * W
    D = w1.shape[1]
    NB = N // TM
    NT = D // 128
    assert B == 1 and dw.shape[:2] == (1, 1) and C == 384 and D == 4 * C and N % TM == 0 and NB > NX
    assert all(a.dtype == BF16 for a in (x, dw, w1, w2))
    hbm = pl.BlockSpec(memory_space=pl.ANY)
    vmem = pl.BlockSpec(memory_space=pltpu.VMEM)
    out, _ = pl.pallas_call(
        _kernel,
        in_specs=[hbm, hbm, hbm, hbm, vmem, vmem],
        out_specs=[hbm, hbm],
        out_shape=[
            jax.ShapeDtypeStruct((N, C), x.dtype),
            jax.ShapeDtypeStruct((NB - NH, NT, TH, 128), BF16),
        ],
        scratch_shapes=[
            pltpu.VMEM((NX, TM, C), BF16),
            pltpu.VMEM((NH, NT, TH, 128), BF16),
            pltpu.VMEM((NB, NT, TC, 128), BF16),
            pltpu.VMEM((15, NT // 3, 64, 128), U32),
            pltpu.VMEM((NL, 15, US, 128), BF16),
            pltpu.VMEM((ND, NL * US, 128), F32),
            pltpu.VMEM((8, D), F32),
            pltpu.VMEM((1, C), BF16),
            pltpu.VMEM((8, C), F32),
            pltpu.VMEM((3, D, 128), BF16),
            pltpu.SemaphoreType.DMA((NX,)),
            pltpu.SemaphoreType.DMA((NH,)),
            pltpu.SemaphoreType.DMA((2,)),
        ],
        compiler_params=pltpu.CompilerParams(
            vmem_limit_bytes=128 * 1024 * 1024, disable_bounds_checks=True),
    )(x.reshape(N, C), dw.reshape(1, C), w1, w2, grn_g, grn_b)
    return out.reshape(x.shape)
```
